```python
import jax
import jax.numpy as jnp

def _softmax(x, axis=-1):
    return jax.nn.softmax(x, axis=axis)
def _gelu(x):
    return jax.nn.gelu(x, approximate=True)
def _silu(x):
    return jax.nn.silu(x)
def _sigmoid(x):
    return jax.nn.sigmoid(x)
def _layernorm(x, axis=-1, eps=1e-5):
    m = jnp.mean(x, axis=axis, keepdims=True)
    v = jnp.var(x, axis=axis, keepdims=True)
    return (x - m) / jnp.sqrt(v + eps)
def _scatter_add(tgt, idx, src, axis=0):
    return tgt.at[idx].add(src)
def _segment_sum(src, seg, n):
    return jax.ops.segment_sum(src, seg, n)
class _Rng:
    def __init__(self, key):
        self._k = key
    def _next(self):
        self._k, sub = jax.random.split(self._k)
        return sub
    def normal(self, shape):
        return jax.random.normal(self._next(), shape, dtype=jnp.bfloat16)
    def randint(self, lo, hi, shape):
        return jax.random.randint(self._next(), shape, lo, hi, dtype=jnp.int32)
    def uniform(self, shape, lo=0.0, hi=1.0):
        return jax.random.uniform(self._next(), shape, jnp.bfloat16, lo, hi)
    def permutation(self, n):
        return jax.random.permutation(self._next(), n)


kernel_name = 'standalone__gqa_block_cached__near_ridge'

def setup_inputs():
    _rng = _Rng(jax.random.key(int.from_bytes(__import__("os").urandom(4), "little")))
    _w = (lambda a: (lambda t: t.astype(jnp.bfloat16) if jnp.issubdtype(t.dtype, jnp.floating) else t)(jnp.asarray(a)))
    B, Sq, D = 16, 240, 640
    Hq, Hkv, Sk, Dh = 32, 32, 1024, 128
    assert Hq % Hkv == 0, (Hq, Hkv)
    return {
        "x": _w((lambda *s: _rng.normal(s) * 0.05)(B, Sq, D)),
        "k_cache": _w((lambda *s: _rng.normal(s) * 0.05)(B, Hkv, Sk, Dh)),
        "v_cache": _w((lambda *s: _rng.normal(s) * 0.05)(B, Hkv, Sk, Dh)),
        "wq": _w((lambda *s: _rng.normal(s) * 0.05)(D, Hq * Dh) * (D ** -0.5)),
        "wo": _w((lambda *s: _rng.normal(s) * 0.05)(Hq * Dh, D) * ((Hq * Dh) ** -0.5)),
    }

def reference(x, k_cache, v_cache, wq, wo):
    B, Sq, D = x.shape
    Hq, Dh = 32, 128
    Hkv = k_cache.shape[1]
    rep = Hq // Hkv
    q = (lambda x, *d: x.transpose(*d))((x @ wq).reshape(B, Sq, Hq, Dh), 0, 2, 1, 3)
    k = jnp.repeat(k_cache, rep, axis=1)
    v = jnp.repeat(v_cache, rep, axis=1)
    scores = jnp.einsum("bhqd,bhkd->bhqk", q, k) * (Dh ** -0.5)
    p = _softmax(scores, axis=-1)
    o = jnp.einsum("bhqk,bhkd->bhqd", p, v)
    return (lambda x, *d: x.transpose(*d))(o, 0, 2, 1, 3).reshape(B, Sq, Hq * Dh) @ wo
```

```python
import functools
import jax
import jax.numpy as jnp
from jax.experimental import pallas as pl
from jax.experimental.pallas import tpu as pltpu

LOG2E = 1.4426950408889634
NT = (((1,), (1,)), ((), ()))
f32 = jnp.float32
bf16 = jnp.bfloat16
GS = 4

SCHED = {
    "s8a": "QK0 QK1 PV0 QK2 PV1 QK3 OPp PV2 QK4 PV3 QP0 QK5 PV4 QK6 PV5 QK7 OP0 PV6 PV7 QP1",
    "s8b": "QK0 QK1 PV0 QK2 PV1 QK3 PV2 QK4 OPp PV3 QP0 QK5 PV4 QK6 PV5 QK7 PV6 OP0 PV7 QP1",
    "s8c": "QK0 QK1 PV0 QK2 PV1 QK3 PV2 QK4 PV3 OPp QK5 PV4 QP0 QK6 PV5 QK7 OP0 PV6 PV7 QP1",
    "s4a": "QK0 QK1 PV0 QK2 PV1 QK3 OPp PV2 PV3 QP0",
    "s4b": "QK0 QK1 PV0 QK2 PV1 QK3 PV2 OPp PV3 QP0",
    "s16a": "QK0 QK1 PV0 QK2 PV1 QK3 OPp PV2 QK4 PV3 QP0 QK5 PV4 QK6 PV5 QK7 OP0 PV6 QK8 PV7 QP1 QK9 PV8 QK10 PV9 QK11 OP1 PV10 QK12 PV11 QP2 QK13 PV12 QK14 PV13 QK15 OP2 PV14 PV15 QP3",
}


def _build(hb=16, sched="s16a", newton=True):
    def fn(x, k_cache, v_cache, wq, wo):
        B, Sq, D = x.shape
        _, H, Sk, Dh = k_cache.shape
        U = hb
        G = H // U
        T = B * G
        NG = U // GS
        c = (Dh ** -0.5) * LOG2E
        nt = Sk // Dh
        W = GS * Dh

        def lax_rem(a, b):
            return jax.lax.rem(a, jnp.int32(b))

        def kernel(xn_ref, k_ref, v_ref, wq_ref, wo_ref, o_ref, acc_ref, q_scr, o_scr, l_scr):
            t = pl.program_id(0)
            g = lax_rem(t, G)
            off_cur = pl.multiple_of(g * (U * Dh), Dh)
            off_next = pl.multiple_of(lax_rem(g + 1, G) * (U * Dh), Dh)
            off_prev = pl.multiple_of(lax_rem(g + (G - 1), G) * (U * Dh) + (U - GS) * Dh, Dh)

            def qp(off, gi):
                q = jnp.dot(xn_ref[0], wq_ref[:, pl.ds(off, W)], preferred_element_type=f32)
                q_scr[gi] = (q * c).astype(bf16)

            @pl.when(t == 0)
            def _():
                acc_ref[...] = jnp.zeros_like(acc_ref)
                o_scr[...] = jnp.zeros_like(o_scr)
                l_scr[...] = jnp.ones_like(l_scr)
                for gi in range(NG):
                    qp(gi * W, gi)

            def qk(h):
                q = q_scr[h // GS, :, (h % GS) * Dh:(h % GS + 1) * Dh]
                return jax.lax.dot_general(q, k_ref[0, h], NT, preferred_element_type=f32)

            def sm(s):
                m = jnp.max(s, axis=-1, keepdims=True)
                p = jnp.exp2(s - m)
                ps = [p[:, j * 128:(j + 1) * 128] for j in range(nt)]
                part = ps[0]
                for j in range(1, nt):
                    part = part + ps[j]
                    if j == 3 or j == nt - 1:
                        ps[j] = jnp.minimum(ps[j], part)
                pb = jnp.concatenate(ps, axis=-1).astype(bf16)
                return pb, part

            def norm(o, part):
                l = jnp.sum(part, axis=-1, keepdims=True)
                inv = pl.reciprocal(l, approx=True)
                if newton:
                    inv = inv * (2.0 - l * inv)
                return o * inv

            def op(ons, woff):
                o_all = jnp.concatenate(ons, axis=-1).astype(bf16)
                return jnp.dot(o_all, wo_ref[pl.ds(woff, W), :], preferred_element_type=f32)

            ss, res = {}, {}
            for item in SCHED[sched].split():
                kind, arg = item[:2], item[2:]
                if kind == "QK":
                    ss[int(arg)] = qk(int(arg))
                elif kind == "PV":
                    h = int(arg)
                    pb, part = sm(ss.pop(h))
                    o = jnp.dot(pb, v_ref[0, h], preferred_element_type=f32)
                    if h >= U - GS:
                        o_scr[h - (U - GS)] = o
                        l_scr[h - (U - GS)] = part
                    else:
                        res[h] = (o, part)
                elif kind == "QP":
                    gi = int(arg)
                    qp(off_next + gi * W, gi)
                elif kind == "OP":
                    if arg == "p":
                        a = acc_ref[...] + op([norm(o_scr[i], l_scr[i]) for i in range(GS)], off_prev)
                        o_ref[0] = a.astype(o_ref.dtype)
                        acc_ref[...] = jnp.where(g == 0, 0.0, a)
                    else:
                        gi = int(arg)
                        acc_ref[...] += op([norm(*res.pop(gi * GS + i)) for i in range(GS)], off_cur + gi * W)

            @pl.when(t == T - 1)
            def _():
                a = acc_ref[...] + op([norm(o_scr[i], l_scr[i]) for i in range(GS)], off_cur + (U - GS) * Dh)
                o_ref[0] = a.astype(o_ref.dtype)

        return pl.pallas_call(
            kernel,
            grid=(T,),
            in_specs=[
                pl.BlockSpec((1, Sq, D), lambda t: (jnp.minimum((t + 1) // G, B - 1), 0, 0)),
                pl.BlockSpec((1, U, Sk, Dh), lambda t: (t // G, t % G, 0, 0)),
                pl.BlockSpec((1, U, Sk, Dh), lambda t: (t // G, t % G, 0, 0)),
                pl.BlockSpec((D, H * Dh), lambda t: (0, 0)),
                pl.BlockSpec((H * Dh, D), lambda t: (0, 0)),
            ],
            out_specs=pl.BlockSpec((1, Sq, D), lambda t: (jnp.maximum(t - 1, 0) // G, 0, 0)),
            out_shape=jax.ShapeDtypeStruct((B, Sq, D), x.dtype),
            scratch_shapes=[pltpu.VMEM((Sq, D), f32),
                            pltpu.VMEM((NG, Sq, W), bf16),
                            pltpu.VMEM((GS, Sq, Dh), f32),
                            pltpu.VMEM((GS, Sq, Dh), f32)],
            compiler_params=pltpu.CompilerParams(
                dimension_semantics=("arbitrary",),
                vmem_limit_bytes=100 * 1024 * 1024,
            ),
        )(x, k_cache, v_cache, wq, wo)

    return fn


@jax.jit
def pallas_standalone__gqa_block_cached__near_ridge_kernel(x, k_cache, v_cache, wq, wo):
    return _build()(x, k_cache, v_cache, wq, wo)
```

```python
import jax
import jax.numpy as jnp
from jax.experimental import pallas as pl
from jax.experimental.pallas import tpu as pltpu

LOG2E = 1.4426950408889634
NT = (((1,), (1,)), ((), ()))
f32 = jnp.float32
bf16 = jnp.bfloat16
GS = 4
UM = 16
NFINE = 12


def _schedule(ng):
    if ng == 1:
        return "QK0 QK1 OPp PV0 QK2 PV1 QK3 PV2 PV3 QPn".split()
    s = ["QK0"]
    for i in range(ng):
        a = GS * i
        last = i == ng - 1
        s += [f"QK{a + 1}", f"PV{a}", f"QK{a + 2}", f"PV{a + 1}"]
        if not last:
            s += [f"QP{i + 1}"]
        s += [f"QK{a + 3}"]
        s += ["OPp"] if i == 0 else [f"OP{i - 1}"]
        s += [f"PV{a + 2}"]
        if not last:
            s += [f"QK{a + 4}"]
        s += [f"PV{a + 3}"]
    s += ["QPn"]
    return s


def _rem(a, b):
    assert b & (b - 1) == 0
    return a % b if isinstance(a, int) else jax.lax.bitwise_and(a, jnp.int32(b - 1))


def _div(a, b):
    assert b & (b - 1) == 0
    return a // b if isinstance(a, int) else jax.lax.shift_right_logical(a, jnp.int32(b.bit_length() - 1))


@jax.jit
def pallas_standalone__gqa_block_cached__near_ridge_kernel(x, k_cache, v_cache, wq, wo):
    B, Sq, D = x.shape
    _, H, Sk, Dh = k_cache.shape
    assert wq.shape == (D, H * Dh) and wo.shape == (H * Dh, D)
    NW = H // GS
    NGM = UM // GS
    NGR = B * NW
    NF = NFINE
    assert NF > NW and NF % NGM == 0 and (NGR - NF) % NGM == 0 and NW % NGM == 0
    NM = (NGR - NF) // NGM
    T = NF + NM + 1
    PD = NGM
    X1S = NW - 1 - PD
    assert 0 <= X1S
    c = (Dh ** -0.5) * LOG2E
    nt = Sk // Dh
    W = GS * Dh
    kf = k_cache.reshape(B * H, Sk, Dh)
    vf = v_cache.reshape(B * H, Sk, Dh)

    def kernel(x_hbm, k_hbm, v_hbm, wq_hbm, wo_hbm, o_ref,
               acc_ref, q_scr, o_scr, l_scr, x_buf, k_buf, v_buf, wq_buf, wo_buf,
               sem_fk, sem_fv, sem_mk, sem_mv, sem_wq, sem_wo, sem_x):
        t = pl.program_id(0)

        def kv_copy(gam, n, fine):
            h0 = gam * GS
            sl = _rem(_div(gam, NGM), 2)
            if n == NGM:
                kd, vd = k_buf.at[sl], v_buf.at[sl]
            else:
                s0 = _rem(h0, UM)
                if not isinstance(s0, int):
                    s0 = pl.multiple_of(s0, GS)
                kd, vd = k_buf.at[sl, pl.ds(s0, n * GS)], v_buf.at[sl, pl.ds(s0, n * GS)]
            if fine:
                i = _rem(gam, 2 * NGM)
                sk, sv = sem_fk.at[i], sem_fv.at[i]
            else:
                i = _rem(_div(gam - NF, NGM), 2)
                sk, sv = sem_mk.at[i], sem_mv.at[i]
            return (pltpu.make_async_copy(k_hbm.at[pl.ds(h0, n * GS)], kd, sk),
                    pltpu.make_async_copy(v_hbm.at[pl.ds(h0, n * GS)], vd, sv))

        def wq_copy(gi):
            return pltpu.make_async_copy(wq_hbm.at[:, pl.ds(gi * W, W)], wq_buf.at[gi], sem_wq.at[gi])

        def wo_copy(gi):
            return pltpu.make_async_copy(wo_hbm.at[pl.ds(gi * W, W), :], wo_buf.at[gi], sem_wo.at[gi])

        def x_copy(b):
            return pltpu.make_async_copy(x_hbm.at[b], x_buf.at[b], sem_x.at[_rem(b, 2)])

        def x_sync(g0, ng):
            b = _div(g0, NW)

            @pl.when(jnp.logical_and(_rem(g0, NW) == 0, b + 2 < B))
            def _():
                x_copy(b + 2).start()

            @pl.when(jnp.logical_and(_rem(g0 + ng, NW) == 0, b + 1 < B))
            def _():
                x_copy(b + 1).wait()

        def softmax_unnorm(s):
            m = jnp.max(s, axis=-1, keepdims=True)
            p = jnp.exp2(s - m)
            ps = [p[:, j * 128:(j + 1) * 128] for j in range(nt)]
            part = ps[0]
            for j in range(1, nt):
                part = part + ps[j]
                if j == 3 or j == nt - 1:
                    ps[j] = jnp.minimum(ps[j], part)
            return jnp.concatenate(ps, axis=-1).astype(bf16), part

        def normalize(o, part):
            l = jnp.sum(part, axis=-1, keepdims=True)
            inv = pl.reciprocal(l, approx=True)
            inv = inv * (2.0 - l * inv)
            return o * inv

        def q_proj(b, gw, slot):
            q = jnp.dot(x_buf[b], wq_buf[gw], preferred_element_type=f32)
            q_scr[slot] = (q * c).astype(bf16)

        def o_proj(ons, gw):
            o_all = jnp.concatenate(ons, axis=-1).astype(bf16)
            return jnp.dot(o_all, wo_buf[gw], preferred_element_type=f32)

        def body(g0, ng):
            b = _div(g0, NW)
            gw0 = _rem(g0, NW)
            gprev = _rem(jnp.maximum(g0 - 1, 0), NW)
            gn = g0 + ng
            gnext = _rem(gn, NW)
            bnext = jnp.minimum(_div(gn, NW), B - 1)
            sl = _rem(_div(g0, NGM), 2)
            s0 = 0 if ng == NGM else pl.multiple_of(_rem(g0 * GS, UM), GS)
            U = ng * GS
            ss, res = {}, {}
            for item in _schedule(ng):
                kind, arg = item[:2], item[2:]
                if kind == "QK":
                    h = int(arg)
                    q = q_scr[h // GS, :, (h % GS) * Dh:(h % GS + 1) * Dh]
                    ss[h] = jax.lax.dot_general(q, k_buf[sl, s0 + h], NT, preferred_element_type=f32)
                elif kind == "PV":
                    h = int(arg)
                    pb, part = softmax_unnorm(ss.pop(h))
                    o = jnp.dot(pb, v_buf[sl, s0 + h], preferred_element_type=f32)
                    if h >= U - GS:
                        o_scr[h - (U - GS)] = o
                        l_scr[h - (U - GS)] = part
                    else:
                        res[h] = (o, part)
                elif kind == "QP":
                    if arg == "n":
                        q_proj(bnext, gnext, 0)
                    else:
                        q_proj(b, gw0 + int(arg), int(arg))
                elif arg == "p":
                    a = acc_ref[...] + o_proj([normalize(o_scr[j], l_scr[j]) for j in range(GS)], gprev)
                    o_ref[0] = a.astype(o_ref.dtype)
                    acc_ref[...] = jnp.where(gw0 == 0, 0.0, a)
                else:
                    i = int(arg)
                    acc_ref[...] += o_proj([normalize(*res.pop(i * GS + j)) for j in range(GS)], gw0 + i)

        @pl.when(t < 1)
        def _():
            x_copy(0).start()
            wq_copy(0).start()

        @pl.when(t == 0)
        def _():
            for gi in range(PD):
                ck, cv = kv_copy(gi, 1, True)
                ck.start()
                cv.start()
                wq_copy(gi + 1).start()
                if gi == 0:
                    wo_copy(0).start()
                elif gi >= 2:
                    wo_copy(gi - 1).start()
            acc_ref[...] = jnp.zeros_like(acc_ref)
            o_scr[...] = jnp.zeros_like(o_scr)
            l_scr[...] = jnp.ones_like(l_scr)
            x_copy(0).wait()
            wq_copy(0).wait()
            q_proj(0, 0, 0)

        @pl.when(t < NF)
        def _():
            g0 = t
            gp = g0 + PD

            @pl.when(gp < NF)
            def _():
                ck, cv = kv_copy(gp, 1, True)
                ck.start()
                cv.start()

            @pl.when(gp >= NF)
            def _():
                ck, cv = kv_copy(gp, 1, False)
                ck.start()
                cv.start()

            @pl.when(gp + 1 < NW)
            def _():
                wq_copy(gp + 1).start()

            @pl.when(gp <= NW)
            def _():
                wo_copy(gp - 1).start()

            @pl.when(g0 == X1S)
            def _():
                x_copy(1).start()

            x_sync(g0, 1)

            @pl.when(g0 + 1 < NW)
            def _():
                wq_copy(g0 + 1).wait()

            @pl.when(jnp.logical_and(g0 <= NW, g0 != 1))
            def _():
                wo_copy(jnp.maximum(g0 - 1, 0)).wait()

            ck, cv = kv_copy(g0, 1, True)
            ck.wait()
            cv.wait()
            body(g0, 1)

        @pl.when(jnp.logical_and(t >= NF, t < T - 1))
        def _():
            g0 = NF + (t - NF) * NGM

            @pl.when(g0 + NGM < NGR)
            def _():
                ck, cv = kv_copy(g0 + NGM, NGM, False)
                ck.start()
                cv.start()

            x_sync(g0, NGM)
            ck, cv = kv_copy(g0, NGM, False)
            ck.wait()
            cv.wait()
            body(g0, NGM)

        @pl.when(t == T - 1)
        def _():
            a = acc_ref[...] + o_proj([normalize(o_scr[j], l_scr[j]) for j in range(GS)], NW - 1)
            o_ref[0] = a.astype(o_ref.dtype)

    def out_index(t):
        g0 = jnp.where(t < NF, t, NF + (t - NF) * NGM)
        return (jnp.minimum(_div(jnp.maximum(g0 - 1, 0), NW), B - 1), 0, 0)

    assert PD + 1 <= NW and PD >= 2
    any_spec = pl.BlockSpec(memory_space=pl.ANY)
    return pl.pallas_call(
        kernel,
        grid=(T,),
        in_specs=[any_spec] * 5,
        out_specs=pl.BlockSpec((1, Sq, D), out_index),
        out_shape=jax.ShapeDtypeStruct((B, Sq, D), x.dtype),
        scratch_shapes=[
            pltpu.VMEM((Sq, D), f32),
            pltpu.VMEM((NGM, Sq, W), bf16),
            pltpu.VMEM((GS, Sq, Dh), f32),
            pltpu.VMEM((GS, Sq, Dh), f32),
            pltpu.VMEM((B, Sq, D), bf16),
            pltpu.VMEM((2, UM, Sk, Dh), bf16),
            pltpu.VMEM((2, UM, Sk, Dh), bf16),
            pltpu.VMEM((NW, D, W), bf16),
            pltpu.VMEM((NW, W, D), bf16),
            pltpu.SemaphoreType.DMA((2 * NGM,)),
            pltpu.SemaphoreType.DMA((2 * NGM,)),
            pltpu.SemaphoreType.DMA((2,)),
            pltpu.SemaphoreType.DMA((2,)),
            pltpu.SemaphoreType.DMA((NW,)),
            pltpu.SemaphoreType.DMA((NW,)),
            pltpu.SemaphoreType.DMA((2,)),
        ],
        compiler_params=pltpu.CompilerParams(
            dimension_semantics=("arbitrary",),
            vmem_limit_bytes=100 * 1024 * 1024,
            disable_bounds_checks=True,
        ),
        name="gqa_block_cached",
    )(x, kf, vf, wq, wo)
```

```python
import jax
import jax.numpy as jnp
from jax.experimental import pallas as pl
from jax.experimental.pallas import tpu as pltpu

LOG2E = 1.4426950408889634
NT = (((1,), (1,)), ((), ()))
f32 = jnp.float32
bf16 = jnp.bfloat16
GS = 4
HS = 16


def _schedule(ng):
    if ng == 1:
        return "QK0 OPp QK1 PV0 QK2 PV1 QK3 PV2 PV3 QPn".split()
    s = []
    ngs = HS // GS
    for i in range(ng):
        a = GS * i
        slot_first = i % ngs == 0
        slot_last = i % ngs == ngs - 1
        if slot_first:
            if i > 0:
                s += ["SY"]
            s += [f"QK{a}"]
        s += [f"QK{a + 1}", f"PV{a}", f"QK{a + 2}", f"PV{a + 1}"]
        if not slot_last:
            s += [f"QP{i + 1}"]
        s += [f"QK{a + 3}", f"PV{a + 2}"]
        s += ["OPp"] if i == 0 else [f"OP{i - 1}"]
        if not slot_last:
            s += [f"QK{a + 4}"]
        s += [f"PV{a + 3}"]
        if slot_last and i != ng - 1:
            s += [f"QP{i + 1}"]
    s += ["QPn"]
    return s


def _rem(a, b):
    assert b & (b - 1) == 0
    return a % b if isinstance(a, int) else jax.lax.bitwise_and(a, jnp.int32(b - 1))


def _div(a, b):
    assert b & (b - 1) == 0
    return a // b if isinstance(a, int) else jax.lax.shift_right_logical(a, jnp.int32(b.bit_length() - 1))


@jax.jit
def pallas_standalone__gqa_block_cached__near_ridge_kernel(x, k_cache, v_cache, wq, wo):
    B, Sq, D = x.shape
    _, H, Sk, Dh = k_cache.shape
    assert wq.shape == (D, H * Dh) and wo.shape == (H * Dh, D)
    assert H == 2 * HS and B >= 4 and Dh == 128
    NW = H // GS
    NGS = HS // GS
    NF = 2 * NW
    NM = B - 2
    T = NF + NM + 1
    PD = NGS
    X2S = NW
    c = (Dh ** -0.5) * LOG2E
    nt = Sk // Dh
    W = GS * Dh
    kf = k_cache.reshape(B * H, Sk, Dh)
    vf = v_cache.reshape(B * H, Sk, Dh)

    def kernel(x_hbm, k_hbm, v_hbm, wq_hbm, wo_hbm, o_ref,
               acc_ref, q_scr, o_scr, l_scr, x_buf, k_buf, v_buf, wq_buf, wo_buf,
               sem_fk, sem_fv, sem_mk, sem_mv, sem_wq, sem_wo, sem_x):
        t = pl.program_id(0)

        def kv_group_copy(gam, fine):
            if isinstance(gam, int):
                h0 = (gam & 1) * H + (gam >> 1) * GS if gam < NF else gam * GS
            else:
                h0 = jnp.where(gam < NF, _rem(gam, 2) * H + _div(gam, 2) * GS, gam * GS)
            sl = _rem(_div(gam, NGS), 2)
            s0 = _rem(gam * GS, HS)
            if not isinstance(s0, int):
                s0 = pl.multiple_of(s0, GS)
            kd, vd = k_buf.at[sl, pl.ds(s0, GS)], v_buf.at[sl, pl.ds(s0, GS)]
            if fine:
                i = _rem(gam, 2 * NGS)
                sk, sv = sem_fk.at[i], sem_fv.at[i]
            else:
                sk, sv = sem_mk.at[sl], sem_mv.at[sl]
            return (pltpu.make_async_copy(k_hbm.at[pl.ds(h0, GS)], kd, sk),
                    pltpu.make_async_copy(v_hbm.at[pl.ds(h0, GS)], vd, sv))

        def k_slot_copy(b, sl):
            return pltpu.make_async_copy(k_hbm.at[pl.ds(b * H + sl * HS, HS)], k_buf.at[sl], sem_mk.at[sl])

        def v_slot_copy(b, sl):
            return pltpu.make_async_copy(v_hbm.at[pl.ds(b * H + sl * HS, HS)], v_buf.at[sl], sem_mv.at[sl])

        def wq_copy(gi):
            return pltpu.make_async_copy(wq_hbm.at[:, pl.ds(gi * W, W)], wq_buf.at[gi], sem_wq.at[gi])

        def wo_copy(gi):
            return pltpu.make_async_copy(wo_hbm.at[pl.ds(gi * W, W), :], wo_buf.at[gi], sem_wo.at[gi])

        def x_copy(b):
            return pltpu.make_async_copy(x_hbm.at[b], x_buf.at[b], sem_x.at[_rem(b, 2)])

        def softmax_unnorm(s):
            m = jnp.max(s, axis=-1, keepdims=True)
            p = jnp.exp2(s - m)
            ps = [p[:, j * 128:(j + 1) * 128] for j in range(nt)]
            part = ps[0]
            for j in range(1, nt):
                part = part + ps[j]
                if j == 3 or j == nt - 1:
                    ps[j] = jnp.minimum(ps[j], part)
            return jnp.concatenate(ps, axis=-1).astype(bf16), part

        def normalize(o, part):
            l = jnp.sum(part, axis=-1, keepdims=True)
            inv = pl.reciprocal(l, approx=True)
            inv = inv * (2.0 - l * inv)
            return o * inv

        def q_proj(b, gw, slot):
            q = jnp.dot(x_buf[b], wq_buf[gw], preferred_element_type=f32)
            q_scr[slot] = (q * c).astype(bf16)

        def o_proj(ons, gw):
            o_all = jnp.concatenate(ons, axis=-1).astype(bf16)
            return jnp.dot(o_all, wo_buf[gw], preferred_element_type=f32)

        def body(g0, ng):
            big = ng == NW
            if big:
                b = _div(g0, NW)
                gprev, gnext = NW - 1, 0
                bnext = jnp.minimum(b + 1, B - 1)
                acc = acc_ref.at[1]
            else:
                gn = g0 + 1
                gprev = _rem(_div(g0 + (2 * NW - 1), 2), NW)
                gnext = jnp.where(gn < NF, _div(gn, 2), 0)
                bnext = jnp.where(gn < NF, _rem(gn, 2), 2)
                sl = _rem(_div(g0, NGS), 2)
                s0 = pl.multiple_of(_rem(g0 * GS, HS), GS)
                acc = acc_ref.at[_rem(g0 + 1, 2)]

            def kv_at(buf, h):
                return buf[h // HS, h % HS] if big else buf[sl, s0 + h]

            U = ng * GS
            nq = q_scr.shape[0]
            ss, res = {}, {}
            acc_fresh = False
            for item in _schedule(ng):
                kind, arg = item[:2], item[2:]
                if kind == "QK":
                    h = int(arg)
                    q = q_scr[(h // GS) % nq, :, (h % GS) * Dh:(h % GS + 1) * Dh]
                    ss[h] = jax.lax.dot_general(q, kv_at(k_buf, h), NT, preferred_element_type=f32)
                elif kind == "PV":
                    h = int(arg)
                    pb, part = softmax_unnorm(ss.pop(h))
                    o = jnp.dot(pb, kv_at(v_buf, h), preferred_element_type=f32)
                    if h >= U - GS:
                        o_scr[h - (U - GS)] = o
                        l_scr[h - (U - GS)] = part
                    else:
                        res[h] = (o, part)
                elif kind == "QP":
                    if arg == "n":
                        q_proj(bnext, gnext, 0)
                    else:
                        q_proj(b, int(arg), int(arg) % nq)
                elif kind == "SY":
                    k_slot_copy(b, 1).wait()
                    v_slot_copy(b, 1).wait()

                    @pl.when(b + 2 < B)
                    def _():
                        x_copy(b + 2).start()

                    @pl.when(b + 1 < B)
                    def _():
                        k_slot_copy(b + 1, 0).start()
                        v_slot_copy(b + 1, 0).start()
                elif arg == "p":
                    a = acc[...] + o_proj([normalize(o_scr[j], l_scr[j]) for j in range(GS)], gprev)
                    o_ref[0] = a.astype(o_ref.dtype)
                    if big:
                        acc_fresh = True
                    else:
                        acc[...] = a
                else:
                    i = int(arg)
                    r = o_proj([normalize(*res.pop(i * GS + j)) for j in range(GS)], i)
                    if acc_fresh:
                        acc[...] = r
                        acc_fresh = False
                    else:
                        acc[...] += r

        @pl.when(t < 1)
        def _():
            x_copy(0).start()
            wq_copy(0).start()
            x_copy(1).start()

        @pl.when(t == 0)
        def _():
            for gi in range(PD):
                ck, cv = kv_group_copy(gi, True)
                ck.start()
                cv.start()
                if gi % 2 == 1:
                    wq_copy((gi + 1) // 2).start()
                    wo_copy((gi - 1) // 2).start()
            acc_ref[...] = jnp.zeros_like(acc_ref)
            o_scr[...] = jnp.zeros_like(o_scr)
            l_scr[...] = jnp.ones_like(l_scr)
            wo_buf[NW - 1] = jnp.zeros((W, D), bf16)
            x_copy(0).wait()
            wq_copy(0).wait()
            q_proj(0, 0, 0)

        @pl.when(t < NF)
        def _():
            g0 = t
            gp = g0 + PD

            @pl.when(gp < NF)
            def _():
                ck, cv = kv_group_copy(gp, True)
                ck.start()
                cv.start()

            @pl.when(gp >= NF)
            def _():
                ck, cv = kv_group_copy(gp, False)
                ck.start()
                cv.start()

            gp_odd = jnp.logical_and(_rem(gp, 2) == 1, gp < NF)

            @pl.when(jnp.logical_and(gp_odd, gp + 1 < NF))
            def _():
                wq_copy(_div(gp + 1, 2)).start()

            @pl.when(gp_odd)
            def _():
                wo_copy(_div(gp - 1, 2)).start()

            @pl.when(g0 == X2S)
            def _():
                x_copy(2).start()

            @pl.when(g0 == X2S + 2)
            def _():
                x_copy(3).start()

            @pl.when(g0 == NF - 1)
            def _():
                x_copy(2).wait()

            @pl.when(g0 == 0)
            def _():
                x_copy(1).wait()

            g_odd = _rem(g0, 2) == 1

            @pl.when(jnp.logical_and(g_odd, g0 + 1 < NF))
            def _():
                wq_copy(_div(g0 + 1, 2)).wait()

            @pl.when(g_odd)
            def _():
                wo_copy(_div(g0 - 1, 2)).wait()

            ck, cv = kv_group_copy(g0, True)
            ck.wait()
            cv.wait()
            body(g0, 1)

            @pl.when(g0 == NF - 1)
            def _():
                k_slot_copy(2, 1).start()
                v_slot_copy(2, 1).start()

        @pl.when(jnp.logical_and(t >= NF, t < T - 1))
        def _():
            b = 2 + (t - NF)

            @pl.when(b + 1 < B)
            def _():
                x_copy(b + 1).wait()

            k_slot_copy(b, 0).wait()
            v_slot_copy(b, 0).wait()
            body(b * NW, NW)

            @pl.when(b + 1 < B)
            def _():
                k_slot_copy(b + 1, 1).start()
                v_slot_copy(b + 1, 1).start()

        @pl.when(t == T - 1)
        def _():
            a = acc_ref[1] + o_proj([normalize(o_scr[j], l_scr[j]) for j in range(GS)], NW - 1)
            o_ref[0] = a.astype(o_ref.dtype)

    def out_index(t):
        return (jnp.where(t < NF, 0, jnp.minimum(t - NF + 1, B - 1)), 0, 0)

    any_spec = pl.BlockSpec(memory_space=pl.ANY)
    return pl.pallas_call(
        kernel,
        grid=(T,),
        in_specs=[any_spec] * 5,
        out_specs=pl.BlockSpec((1, Sq, D), out_index),
        out_shape=jax.ShapeDtypeStruct((B, Sq, D), x.dtype),
        scratch_shapes=[
            pltpu.VMEM((2, Sq, D), f32),
            pltpu.VMEM((4, Sq, W), bf16),
            pltpu.VMEM((GS, Sq, Dh), f32),
            pltpu.VMEM((GS, Sq, Dh), f32),
            pltpu.VMEM((B, Sq, D), bf16),
            pltpu.VMEM((2, HS, Sk, Dh), bf16),
            pltpu.VMEM((2, HS, Sk, Dh), bf16),
            pltpu.VMEM((NW, D, W), bf16),
            pltpu.VMEM((NW, W, D), bf16),
            pltpu.SemaphoreType.DMA((2 * NGS,)),
            pltpu.SemaphoreType.DMA((2 * NGS,)),
            pltpu.SemaphoreType.DMA((2,)),
            pltpu.SemaphoreType.DMA((2,)),
            pltpu.SemaphoreType.DMA((NW,)),
            pltpu.SemaphoreType.DMA((NW,)),
            pltpu.SemaphoreType.DMA((2,)),
        ],
        compiler_params=pltpu.CompilerParams(
            dimension_semantics=("arbitrary",),
            vmem_limit_bytes=100 * 1024 * 1024,
            disable_bounds_checks=True,
        ),
        name="gqa_block_cached",
    )(x, kf, vf, wq, wo)
```

```python
import jax
import jax.numpy as jnp
from jax.experimental import pallas as pl
from jax.experimental.pallas import tpu as pltpu

LOG2E = 1.4426950408889634
NT = (((1,), (1,)), ((), ()))
f32 = jnp.float32
bf16 = jnp.bfloat16
GS = 4
HS = 16


def _schedule(ng):
    if ng == 1:
        return "QK0 OPp QK1 PV0 QK2 PV1 QK3 PV2 PV3 QPn".split()
    s = []
    ngs = HS // GS
    for i in range(ng):
        a = GS * i
        slot_first = i % ngs == 0
        slot_last = i % ngs == ngs - 1
        if slot_first:
            if i > 0:
                s += ["SY"]
            s += [f"QK{a}"]
        s += [f"QK{a + 1}", f"PV{a}", f"QK{a + 2}", f"PV{a + 1}"]
        if not slot_last:
            s += [f"QP{i + 1}"]
        s += [f"QK{a + 3}", f"PV{a + 2}"]
        s += ["OPp"] if i == 0 else [f"OP{i - 1}"]
        if not slot_last:
            s += [f"QK{a + 4}"]
        s += [f"PV{a + 3}"]
        if slot_last and i != ng - 1:
            s += [f"QP{i + 1}"]
    s += ["QPn"]
    return s


def _rem(a, b):
    assert b & (b - 1) == 0
    return a % b if isinstance(a, int) else jax.lax.bitwise_and(a, jnp.int32(b - 1))


def _div(a, b):
    assert b & (b - 1) == 0
    return a // b if isinstance(a, int) else jax.lax.shift_right_logical(a, jnp.int32(b.bit_length() - 1))


@jax.jit
def pallas_standalone__gqa_block_cached__near_ridge_kernel(x, k_cache, v_cache, wq, wo):
    B, Sq, D = x.shape
    _, H, Sk, Dh = k_cache.shape
    assert wq.shape == (D, H * Dh) and wo.shape == (H * Dh, D)
    assert H == 2 * HS and B >= 4 and Dh == 128
    NW = H // GS
    NGS = HS // GS
    NF = 2 * NW
    NM = B - 2
    T = NF + NM + 1
    PD = NGS + 1
    X2S = NW
    c = (Dh ** -0.5) * LOG2E
    nt = Sk // Dh
    W = GS * Dh
    kf = k_cache.reshape(B * H, Sk, Dh)
    vf = v_cache.reshape(B * H, Sk, Dh)

    def kernel(x_hbm, k_hbm, v_hbm, wq_hbm, wo_hbm, o_ref,
               acc_ref, q_scr, o_scr, l_scr, x_buf, k_buf, v_buf, wq_buf, wo_buf,
               sem_fk, sem_fv, sem_mk, sem_mv, sem_wq, sem_wo, sem_x):
        t = pl.program_id(0)

        def kv_group_copy(gam, fine):
            if isinstance(gam, int):
                h0 = (gam & 1) * H + (gam >> 1) * GS if gam < NF else gam * GS
            else:
                h0 = jnp.where(gam < NF, _rem(gam, 2) * H + _div(gam, 2) * GS, gam * GS)
            sl = _rem(_div(gam, NGS), 2)
            s0 = _rem(gam * GS, HS)
            if not isinstance(s0, int):
                s0 = pl.multiple_of(s0, GS)
            kd, vd = k_buf.at[sl, pl.ds(s0, GS)], v_buf.at[sl, pl.ds(s0, GS)]
            if fine:
                i = _rem(gam, 2 * NGS)
                sk, sv = sem_fk.at[i], sem_fv.at[i]
            else:
                sk, sv = sem_mk.at[sl], sem_mv.at[sl]
            return (pltpu.make_async_copy(k_hbm.at[pl.ds(h0, GS)], kd, sk),
                    pltpu.make_async_copy(v_hbm.at[pl.ds(h0, GS)], vd, sv))

        def k_slot_copy(b, sl):
            return pltpu.make_async_copy(k_hbm.at[pl.ds(b * H + sl * HS, HS)], k_buf.at[sl], sem_mk.at[sl])

        def v_slot_copy(b, sl):
            return pltpu.make_async_copy(v_hbm.at[pl.ds(b * H + sl * HS, HS)], v_buf.at[sl], sem_mv.at[sl])

        def wq_copy(gi):
            return pltpu.make_async_copy(wq_hbm.at[:, pl.ds(gi * W, W)], wq_buf.at[gi], sem_wq.at[gi])

        def wo_copy(gi):
            return pltpu.make_async_copy(wo_hbm.at[pl.ds(gi * W, W), :], wo_buf.at[gi], sem_wo.at[gi])

        def x_copy(b):
            return pltpu.make_async_copy(x_hbm.at[b], x_buf.at[b], sem_x.at[_rem(b, 2)])

        def softmax_unnorm(s):
            m = jnp.max(s, axis=-1, keepdims=True)
            p = jnp.exp2(s - m)
            ps = [p[:, j * 128:(j + 1) * 128] for j in range(nt)]
            part = ps[0]
            for j in range(1, nt):
                part = part + ps[j]
                if j == 3 or j == nt - 1:
                    ps[j] = jnp.minimum(ps[j], part)
            return jnp.concatenate(ps, axis=-1).astype(bf16), part

        def normalize(o, part):
            l = jnp.sum(part, axis=-1, keepdims=True)
            inv = pl.reciprocal(l, approx=True)
            inv = inv * (2.0 - l * inv)
            return o * inv

        def q_proj(b, gw, slot):
            q = jnp.dot(x_buf[b], wq_buf[gw], preferred_element_type=f32)
            q_scr[slot] = (q * c).astype(bf16)

        def o_proj(ons, gw):
            o_all = jnp.concatenate(ons, axis=-1).astype(bf16)
            return jnp.dot(o_all, wo_buf[gw], preferred_element_type=f32)

        def body(g0, ng):
            big = ng == NW
            if big:
                b = _div(g0, NW)
                gprev, gnext = NW - 1, 0
                bnext = jnp.minimum(b + 1, B - 1)
                acc = acc_ref.at[1]
            else:
                gn = g0 + 1
                gprev = _rem(_div(g0 + (2 * NW - 1), 2), NW)
                gnext = jnp.where(gn < NF, _div(gn, 2), 0)
                bnext = jnp.where(gn < NF, _rem(gn, 2), 2)
                sl = _rem(_div(g0, NGS), 2)
                s0 = pl.multiple_of(_rem(g0 * GS, HS), GS)
                acc = acc_ref.at[_rem(g0 + 1, 2)]

            def kv_at(buf, h):
                return buf[h // HS, h % HS] if big else buf[sl, s0 + h]

            U = ng * GS
            nq = q_scr.shape[0]
            ss, res = {}, {}
            acc_fresh = False
            for item in _schedule(ng):
                kind, arg = item[:2], item[2:]
                if kind == "QK":
                    h = int(arg)
                    q = q_scr[(h // GS) % nq, :, (h % GS) * Dh:(h % GS + 1) * Dh]
                    ss[h] = jax.lax.dot_general(q, kv_at(k_buf, h), NT, preferred_element_type=f32)
                elif kind == "PV":
                    h = int(arg)
                    pb, part = softmax_unnorm(ss.pop(h))
                    o = jnp.dot(pb, kv_at(v_buf, h), preferred_element_type=f32)
                    if h >= U - GS:
                        o_scr[h - (U - GS)] = o
                        l_scr[h - (U - GS)] = part
                    else:
                        res[h] = (o, part)
                elif kind == "QP":
                    if arg == "n":
                        q_proj(bnext, gnext, 0)
                    else:
                        q_proj(b, int(arg), int(arg) % nq)
                elif kind == "SY":
                    k_slot_copy(b, 1).wait()
                    v_slot_copy(b, 1).wait()

                    @pl.when(b + 2 < B)
                    def _():
                        x_copy(b + 2).start()

                    @pl.when(b + 1 < B)
                    def _():
                        k_slot_copy(b + 1, 0).start()
                        v_slot_copy(b + 1, 0).start()
                elif arg == "p":
                    a = acc[...] + o_proj([normalize(o_scr[j], l_scr[j]) for j in range(GS)], gprev)
                    o_ref[0] = a.astype(o_ref.dtype)
                    if big:
                        acc_fresh = True
                    else:
                        acc[...] = a
                else:
                    i = int(arg)
                    r = o_proj([normalize(*res.pop(i * GS + j)) for j in range(GS)], i)
                    if acc_fresh:
                        acc[...] = r
                        acc_fresh = False
                    else:
                        acc[...] += r

        @pl.when(t < 1)
        def _():
            x_copy(0).start()
            wq_copy(0).start()
            x_copy(1).start()
            wo_buf[NW - 1] = jnp.zeros((W, D), bf16)

        def first_starts(groups):
            for gi in groups:
                ck, cv = kv_group_copy(gi, True)
                ck.start()
                cv.start()
                if gi % 2 == 1:
                    wq_copy((gi + 1) // 2).start()
                    wo_copy((gi - 1) // 2).start()

        @pl.when(t == 0)
        def _():
            first_starts(range(0, 2))
            acc_ref[...] = jnp.zeros_like(acc_ref)

        @pl.when(t <= 0)
        def _():
            first_starts(range(2, PD))
            o_scr[...] = jnp.zeros_like(o_scr)
            l_scr[...] = jnp.ones_like(l_scr)
            x_copy(0).wait()
            wq_copy(0).wait()
            q_proj(0, 0, 0)

        @pl.when(t < NF)
        def _():
            g0 = t

            @pl.when(g0 == NF - 1)
            def _():
                x_copy(2).wait()

            @pl.when(g0 == 0)
            def _():
                x_copy(1).wait()

            g_odd = _rem(g0, 2) == 1

            @pl.when(jnp.logical_and(g_odd, g0 + 1 < NF))
            def _():
                wq_copy(_div(g0 + 1, 2)).wait()

            @pl.when(g_odd)
            def _():
                wo_copy(_div(g0 - 1, 2)).wait()

            ck, cv = kv_group_copy(g0, True)
            ck.wait()
            cv.wait()
            body(g0, 1)

            gp = g0 + PD

            @pl.when(gp < NF)
            def _():
                ck, cv = kv_group_copy(gp, True)
                ck.start()
                cv.start()

            @pl.when(jnp.logical_and(gp >= NF, gp < NF + NGS))
            def _():
                ck, cv = kv_group_copy(gp, False)
                ck.start()
                cv.start()

            gp_odd = jnp.logical_and(_rem(gp, 2) == 1, gp < NF)

            @pl.when(jnp.logical_and(gp_odd, gp + 1 < NF))
            def _():
                wq_copy(_div(gp + 1, 2)).start()

            @pl.when(gp_odd)
            def _():
                wo_copy(_div(gp - 1, 2)).start()

            @pl.when(g0 == X2S)
            def _():
                x_copy(2).start()

            @pl.when(g0 == X2S + 2)
            def _():
                x_copy(3).start()

            @pl.when(g0 == NF - 1)
            def _():
                k_slot_copy(2, 1).start()
                v_slot_copy(2, 1).start()

        @pl.when(jnp.logical_and(t >= NF, t < T - 1))
        def _():
            b = 2 + (t - NF)

            @pl.when(b + 1 < B)
            def _():
                x_copy(b + 1).wait()

            k_slot_copy(b, 0).wait()
            v_slot_copy(b, 0).wait()
            body(b * NW, NW)

            @pl.when(b + 1 < B)
            def _():
                k_slot_copy(b + 1, 1).start()
                v_slot_copy(b + 1, 1).start()

        @pl.when(t == T - 1)
        def _():
            a = acc_ref[1] + o_proj([normalize(o_scr[j], l_scr[j]) for j in range(GS)], NW - 1)
            o_ref[0] = a.astype(o_ref.dtype)

    def out_index(t):
        return (jnp.where(t < NF, 0, jnp.minimum(t - NF + 1, B - 1)), 0, 0)

    any_spec = pl.BlockSpec(memory_space=pl.ANY)
    return pl.pallas_call(
        kernel,
        grid=(T,),
        in_specs=[any_spec] * 5,
        out_specs=pl.BlockSpec((1, Sq, D), out_index),
        out_shape=jax.ShapeDtypeStruct((B, Sq, D), x.dtype),
        scratch_shapes=[
            pltpu.VMEM((2, Sq, D), f32),
            pltpu.VMEM((4, Sq, W), bf16),
            pltpu.VMEM((GS, Sq, Dh), f32),
            pltpu.VMEM((GS, Sq, Dh), f32),
            pltpu.VMEM((B, Sq, D), bf16),
            pltpu.VMEM((2, HS, Sk, Dh), bf16),
            pltpu.VMEM((2, HS, Sk, Dh), bf16),
            pltpu.VMEM((NW, D, W), bf16),
            pltpu.VMEM((NW, W, D), bf16),
            pltpu.SemaphoreType.DMA((2 * NGS,)),
            pltpu.SemaphoreType.DMA((2 * NGS,)),
            pltpu.SemaphoreType.DMA((2,)),
            pltpu.SemaphoreType.DMA((2,)),
            pltpu.SemaphoreType.DMA((NW,)),
            pltpu.SemaphoreType.DMA((NW,)),
            pltpu.SemaphoreType.DMA((2,)),
        ],
        compiler_params=pltpu.CompilerParams(
            dimension_semantics=("arbitrary",),
            vmem_limit_bytes=100 * 1024 * 1024,
            disable_bounds_checks=True,
        ),
        name="gqa_block_cached",
    )(x, kf, vf, wq, wo)
```

```python
import jax
import jax.numpy as jnp
from jax.experimental import pallas as pl
from jax.experimental.pallas import tpu as pltpu

LOG2E = 1.4426950408889634
NT = (((1,), (1,)), ((), ()))
f32 = jnp.float32
bf16 = jnp.bfloat16
GS = 4
HS = 16


def _schedule(ng):
    if ng == 1:
        return "QP0 QK0 OPp QK1 PV0 QK2 PV1 QK3 PV2 PV3".split()
    s = []
    ngs = HS // GS
    for i in range(ng):
        a = GS * i
        slot_first = i % ngs == 0
        slot_last = i % ngs == ngs - 1
        if slot_first:
            s += ["SY"] if i > 0 else []
            s += [f"QP{i}", f"QK{a}"]
        s += [f"QK{a + 1}", f"PV{a}", f"QK{a + 2}", f"PV{a + 1}"]
        s += [] if slot_last else [f"QP{i + 1}"]
        s += ["OPp"] if i == 0 else [f"OP{i - 1}"]
        s += [f"QK{a + 3}", f"PV{a + 2}"]
        s += [] if slot_last else [f"QK{a + 4}"]
        s += [f"PV{a + 3}"]
    return s


def _rem(a, b):
    assert b & (b - 1) == 0
    return a % b if isinstance(a, int) else jax.lax.bitwise_and(a, jnp.int32(b - 1))


def _div(a, b):
    assert b & (b - 1) == 0
    return a // b if isinstance(a, int) else jax.lax.shift_right_logical(a, jnp.int32(b.bit_length() - 1))


@jax.jit
def pallas_standalone__gqa_block_cached__near_ridge_kernel(x, k_cache, v_cache, wq, wo):
    B, Sq, D = x.shape
    _, H, Sk, Dh = k_cache.shape
    assert wq.shape == (D, H * Dh) and wo.shape == (H * Dh, D)
    assert H == 2 * HS and B >= 4 and Dh == 128
    NW = H // GS
    NGS = HS // GS
    NF = 2 * NW
    NM = B - 2
    T = NF + NM + 1
    PD = NGS + 1
    X2S = NW
    c = (Dh ** -0.5) * LOG2E
    nt = Sk // Dh
    W = GS * Dh
    kf = k_cache.reshape(B * H, Sk, Dh)
    vf = v_cache.reshape(B * H, Sk, Dh)

    def kernel(x_hbm, k_hbm, v_hbm, wq_hbm, wo_hbm, o_ref,
               acc_ref, q_scr, o_scr, l_scr, x_buf, k_buf, v_buf, wq_buf, wo_buf,
               sem_fk, sem_fv, sem_mk, sem_mv, sem_wq, sem_wo, sem_x):
        t = pl.program_id(0)

        def kv_group_copy(gam, fine):
            if isinstance(gam, int):
                h0 = (gam & 1) * H + (gam >> 1) * GS if gam < NF else gam * GS
            else:
                h0 = jnp.where(gam < NF, _rem(gam, 2) * H + _div(gam, 2) * GS, gam * GS)
            sl = _rem(_div(gam, NGS), 2)
            s0 = _rem(gam * GS, HS)
            if not isinstance(s0, int):
                s0 = pl.multiple_of(s0, GS)
            kd, vd = k_buf.at[sl, pl.ds(s0, GS)], v_buf.at[sl, pl.ds(s0, GS)]
            if fine:
                i = _rem(gam, 2 * NGS)
                sk, sv = sem_fk.at[i], sem_fv.at[i]
            else:
                sk, sv = sem_mk.at[sl], sem_mv.at[sl]
            return (pltpu.make_async_copy(k_hbm.at[pl.ds(h0, GS)], kd, sk),
                    pltpu.make_async_copy(v_hbm.at[pl.ds(h0, GS)], vd, sv))

        def k_slot_copy(b, sl):
            return pltpu.make_async_copy(k_hbm.at[pl.ds(b * H + sl * HS, HS)], k_buf.at[sl], sem_mk.at[sl])

        def v_slot_copy(b, sl):
            return pltpu.make_async_copy(v_hbm.at[pl.ds(b * H + sl * HS, HS)], v_buf.at[sl], sem_mv.at[sl])

        def wq_copy(gi):
            return pltpu.make_async_copy(wq_hbm.at[:, pl.ds(gi * W, W)], wq_buf.at[gi], sem_wq.at[gi])

        def wo_copy(gi):
            return pltpu.make_async_copy(wo_hbm.at[pl.ds(gi * W, W), :], wo_buf.at[gi], sem_wo.at[gi])

        def x_copy(b):
            return pltpu.make_async_copy(x_hbm.at[b], x_buf.at[b], sem_x.at[_rem(b, 2)])

        def softmax_unnorm(s):
            m = jnp.max(s, axis=-1, keepdims=True)
            p = jnp.exp2(s - m)
            ps = [p[:, j * 128:(j + 1) * 128] for j in range(nt)]
            part = ps[0]
            for j in range(1, nt):
                part = part + ps[j]
                if j == 3 or j == nt - 1:
                    ps[j] = jnp.minimum(ps[j], part)
            return jnp.concatenate(ps, axis=-1).astype(bf16), part

        def normalize(o, part):
            l = jnp.sum(part, axis=-1, keepdims=True)
            inv = pl.reciprocal(l, approx=True)
            inv = inv * (2.0 - l * inv)
            return o * inv

        def q_proj(b, gw, slot):
            q = jnp.dot(x_buf[b], wq_buf[gw], preferred_element_type=f32)
            q_scr[slot] = (q * c).astype(bf16)

        def o_proj(ons, gw):
            o_all = jnp.concatenate(ons, axis=-1).astype(bf16)
            return jnp.dot(o_all, wo_buf[gw], preferred_element_type=f32)

        def body(g0, ng):
            big = ng == NW
            if big:
                b = _div(g0, NW)
                gprev = NW - 1
                acc = acc_ref.at[1]
            else:
                b = _rem(g0, 2)
                gw = _div(g0, 2)
                gprev = _rem(_div(g0 + (2 * NW - 1), 2), NW)
                sl = _rem(_div(g0, NGS), 2)
                s0 = pl.multiple_of(_rem(g0 * GS, HS), GS)
                acc = acc_ref.at[_rem(g0 + 1, 2)]

            def kv_at(buf, h):
                return buf[h // HS, h % HS] if big else buf[sl, s0 + h]

            U = ng * GS
            nq = q_scr.shape[0]
            ss, res = {}, {}
            acc_fresh = False
            for item in _schedule(ng):
                kind, arg = item[:2], item[2:]
                if kind == "QK":
                    h = int(arg)
                    q = q_scr[(h // GS) % nq, :, (h % GS) * Dh:(h % GS + 1) * Dh]
                    ss[h] = jax.lax.dot_general(q, kv_at(k_buf, h), NT, preferred_element_type=f32)
                elif kind == "PV":
                    h = int(arg)
                    pb, part = softmax_unnorm(ss.pop(h))
                    o = jnp.dot(pb, kv_at(v_buf, h), preferred_element_type=f32)
                    if h >= U - GS:
                        o_scr[h - (U - GS)] = o
                        l_scr[h - (U - GS)] = part
                    else:
                        res[h] = (o, part)
                elif kind == "QP":
                    if big:
                        q_proj(b, int(arg), int(arg) % nq)
                    else:
                        q_proj(b, gw, 0)
                elif kind == "SY":
                    k_slot_copy(b, 1).wait()
                    v_slot_copy(b, 1).wait()

                    @pl.when(b + 2 < B)
                    def _():
                        x_copy(b + 2).start()

                    @pl.when(b + 1 < B)
                    def _():
                        k_slot_copy(b + 1, 0).start()
                        v_slot_copy(b + 1, 0).start()
                elif arg == "p":
                    a = acc[...] + o_proj([normalize(o_scr[j], l_scr[j]) for j in range(GS)], gprev)
                    o_ref[0] = a.astype(o_ref.dtype)
                    if big:
                        acc_fresh = True
                    else:
                        acc[...] = a
                else:
                    i = int(arg)
                    r = o_proj([normalize(*res.pop(i * GS + j)) for j in range(GS)], i)
                    if acc_fresh:
                        acc[...] = r
                        acc_fresh = False
                    else:
                        acc[...] += r

        def first_starts(groups):
            for gi in groups:
                ck, cv = kv_group_copy(gi, True)
                ck.start()
                cv.start()
                if gi == 1:
                    x_copy(1).start()
                if gi % 2 == 1:
                    wo_copy((gi - 1) // 2).start()
                elif gi > 0:
                    wq_copy(gi // 2).start()

        @pl.when(t < 1)
        def _():
            x_copy(0).start()
            wq_copy(0).start()
            wo_buf[NW - 1] = jnp.zeros((W, D), bf16)

        @pl.when(t == 0)
        def _():
            first_starts(range(0, 1))
            acc_ref[0] = jnp.zeros((Sq, D), f32)

        @pl.when(t <= 0)
        def _():
            first_starts(range(1, 3))
            acc_ref[1] = jnp.zeros((Sq, D), f32)

        @pl.when(t + 1 == 1)
        def _():
            first_starts(range(3, PD))
            o_scr[...] = jnp.zeros_like(o_scr)
            l_scr[...] = jnp.ones_like(l_scr)

        @pl.when(t < NF)
        def _():
            g0 = t
            g_odd = _rem(g0, 2) == 1

            @pl.when(g0 < 2)
            def _():
                x_copy(g0).wait()

            @pl.when(jnp.logical_not(g_odd))
            def _():
                wq_copy(_div(g0, 2)).wait()

            @pl.when(g_odd)
            def _():
                wo_copy(_div(g0 - 1, 2)).wait()

            ck, cv = kv_group_copy(g0, True)
            ck.wait()
            cv.wait()
            body(g0, 1)

            gp = g0 + PD

            @pl.when(gp < NF)
            def _():
                ck, cv = kv_group_copy(gp, True)
                ck.start()
                cv.start()

            @pl.when(jnp.logical_and(gp >= NF, gp < NF + NGS))
            def _():
                ck, cv = kv_group_copy(gp, False)
                ck.start()
                cv.start()

            gp_odd = _rem(gp, 2) == 1

            @pl.when(jnp.logical_and(jnp.logical_not(gp_odd), gp < NF))
            def _():
                wq_copy(_div(gp, 2)).start()

            @pl.when(jnp.logical_and(gp_odd, gp < NF))
            def _():
                wo_copy(_div(gp - 1, 2)).start()

            @pl.when(g0 == X2S)
            def _():
                x_copy(2).start()

            @pl.when(g0 == X2S + 2)
            def _():
                x_copy(3).start()

            @pl.when(g0 == NF - 1)
            def _():
                k_slot_copy(2, 1).start()
                v_slot_copy(2, 1).start()

        @pl.when(jnp.logical_and(t >= NF, t < T - 1))
        def _():
            b = 2 + (t - NF)
            x_copy(b).wait()
            k_slot_copy(b, 0).wait()
            v_slot_copy(b, 0).wait()
            body(b * NW, NW)

            @pl.when(b + 1 < B)
            def _():
                k_slot_copy(b + 1, 1).start()
                v_slot_copy(b + 1, 1).start()

        @pl.when(t == T - 1)
        def _():
            a = acc_ref[1] + o_proj([normalize(o_scr[j], l_scr[j]) for j in range(GS)], NW - 1)
            o_ref[0] = a.astype(o_ref.dtype)

    def out_index(t):
        return (jnp.where(t < NF, 0, jnp.minimum(t - NF + 1, B - 1)), 0, 0)

    any_spec = pl.BlockSpec(memory_space=pl.ANY)
    return pl.pallas_call(
        kernel,
        grid=(T,),
        in_specs=[any_spec] * 5,
        out_specs=pl.BlockSpec((1, Sq, D), out_index),
        out_shape=jax.ShapeDtypeStruct((B, Sq, D), x.dtype),
        scratch_shapes=[
            pltpu.VMEM((2, Sq, D), f32),
            pltpu.VMEM((4, Sq, W), bf16),
            pltpu.VMEM((GS, Sq, Dh), f32),
            pltpu.VMEM((GS, Sq, Dh), f32),
            pltpu.VMEM((B, Sq, D), bf16),
            pltpu.VMEM((2, HS, Sk, Dh), bf16),
            pltpu.VMEM((2, HS, Sk, Dh), bf16),
            pltpu.VMEM((NW, D, W), bf16),
            pltpu.VMEM((NW, W, D), bf16),
            pltpu.SemaphoreType.DMA((2 * NGS,)),
            pltpu.SemaphoreType.DMA((2 * NGS,)),
            pltpu.SemaphoreType.DMA((2,)),
            pltpu.SemaphoreType.DMA((2,)),
            pltpu.SemaphoreType.DMA((NW,)),
            pltpu.SemaphoreType.DMA((NW,)),
            pltpu.SemaphoreType.DMA((2,)),
        ],
        compiler_params=pltpu.CompilerParams(
            dimension_semantics=("arbitrary",),
            vmem_limit_bytes=100 * 1024 * 1024,
            disable_bounds_checks=True,
        ),
        name="gqa_block_cached",
    )(x, kf, vf, wq, wo)
```

```python
import jax
import jax.numpy as jnp
from jax.experimental import pallas as pl
from jax.experimental.pallas import tpu as pltpu

LOG2E = 1.4426950408889634
NT = (((1,), (1,)), ((), ()))
f32 = jnp.float32
bf16 = jnp.bfloat16
GS = 4
HS = 16


def _schedule(ng):
    if ng == 1:
        return "QP0 QK0 OPp QK1 PV0 QK2 PV1 QK3 PV2 PV3".split()
    assert ng == 8 and HS == 16 and GS == 4
    extra = [("QP1", "QK3"), ("OPp", "QK4"), ("QP2", "QK7"), ("O20", "QK11"), ("QP3", "QK11"),
             ("O22", "QK19"), ("QP5", "QK19"), ("QP6", "QK23"), ("O24", "QK26"), ("QP7", "QK27"),
             ("O16", "QK30")]
    s = []
    for h0 in (0, HS):
        dots = ["SY"] if h0 else []
        dots += [f"QP{h0 // GS}", f"QK{h0}"]
        for h in range(h0, h0 + HS):
            dots += [f"QK{h + 1}"] if h + 1 < h0 + HS else []
            dots += [f"PV{h}"]
        for d in dots:
            s += [item for item, before in extra if before == d] + [d]
    return s


def _rem(a, b):
    assert b & (b - 1) == 0
    return a % b if isinstance(a, int) else jax.lax.bitwise_and(a, jnp.int32(b - 1))


def _div(a, b):
    assert b & (b - 1) == 0
    return a // b if isinstance(a, int) else jax.lax.shift_right_logical(a, jnp.int32(b.bit_length() - 1))


@jax.jit
def pallas_standalone__gqa_block_cached__near_ridge_kernel(x, k_cache, v_cache, wq, wo):
    B, Sq, D = x.shape
    _, H, Sk, Dh = k_cache.shape
    assert wq.shape == (D, H * Dh) and wo.shape == (H * Dh, D)
    assert H == 2 * HS and B >= 4 and Dh == 128
    NW = H // GS
    NGS = HS // GS
    NF = 2 * NW
    NM = B - 2
    T = NF + NM + 1
    PD = NGS + 1
    X2S = NW
    c = (Dh ** -0.5) * LOG2E
    nt = Sk // Dh
    W = GS * Dh
    kf = k_cache.reshape(B * H, Sk, Dh)
    vf = v_cache.reshape(B * H, Sk, Dh)

    def kernel(x_hbm, k_hbm, v_hbm, wq_hbm, wo_hbm, o_ref,
               acc_ref, q_scr, o_scr, l_scr, x_buf, k_buf, v_buf, wq_buf, wo_buf,
               sem_fk, sem_fv, sem_mk, sem_mv, sem_wq, sem_wo, sem_x):
        t = pl.program_id(0)

        def kv_group_copy(gam, fine):
            if isinstance(gam, int):
                h0 = (gam & 1) * H + (gam >> 1) * GS if gam < NF else gam * GS
            else:
                h0 = jnp.where(gam < NF, _rem(gam, 2) * H + _div(gam, 2) * GS, gam * GS)
            sl = _rem(_div(gam, NGS), 2)
            s0 = _rem(gam * GS, HS)
            if not isinstance(s0, int):
                s0 = pl.multiple_of(s0, GS)
            kd, vd = k_buf.at[sl, pl.ds(s0, GS)], v_buf.at[sl, pl.ds(s0, GS)]
            if fine:
                i = _rem(gam, 2 * NGS)
                sk, sv = sem_fk.at[i], sem_fv.at[i]
            else:
                sk, sv = sem_mk.at[sl], sem_mv.at[sl]
            return (pltpu.make_async_copy(k_hbm.at[pl.ds(h0, GS)], kd, sk),
                    pltpu.make_async_copy(v_hbm.at[pl.ds(h0, GS)], vd, sv))

        def k_slot_copy(b, sl):
            return pltpu.make_async_copy(k_hbm.at[pl.ds(b * H + sl * HS, HS)], k_buf.at[sl], sem_mk.at[sl])

        def v_slot_copy(b, sl):
            return pltpu.make_async_copy(v_hbm.at[pl.ds(b * H + sl * HS, HS)], v_buf.at[sl], sem_mv.at[sl])

        def wq_copy(gi):
            return pltpu.make_async_copy(wq_hbm.at[:, pl.ds(gi * W, W)], wq_buf.at[gi], sem_wq.at[gi])

        def wo_copy(gi):
            return pltpu.make_async_copy(wo_hbm.at[pl.ds(gi * W, W), :], wo_buf.at[gi], sem_wo.at[gi])

        def x_copy(b):
            return pltpu.make_async_copy(x_hbm.at[b], x_buf.at[b], sem_x.at[_rem(b, 2)])

        def softmax_unnorm(s):
            m = jnp.max(s, axis=-1, keepdims=True)
            p = jnp.exp2(s - m)
            ps = [p[:, j * 128:(j + 1) * 128] for j in range(nt)]
            part = ps[0]
            for j in range(1, nt):
                part = part + ps[j]
                if j == 3 or j == nt - 1:
                    ps[j] = jnp.minimum(ps[j], part)
            return jnp.concatenate(ps, axis=-1).astype(bf16), part

        def normalize(o, part):
            l = jnp.sum(part, axis=-1, keepdims=True)
            inv = pl.reciprocal(l, approx=True)
            inv = inv * (2.0 - l * inv)
            return o * inv

        def q_proj(b, gw, slot):
            q = jnp.dot(x_buf[b], wq_buf[gw], preferred_element_type=f32)
            q_scr[slot] = (q * c).astype(bf16)

        def o_proj(ons, gw):
            n = len(ons) // GS
            o_all = jnp.concatenate(ons, axis=-1).astype(bf16)
            w = wo_buf[gw] if n == 1 else wo_buf[pl.ds(gw, n)].reshape(n * W, D)
            return jnp.dot(o_all, w, preferred_element_type=f32)

        def body(g0, ng):
            big = ng == NW
            if big:
                b = _div(g0, NW)
                gprev = NW - 1
                acc = acc_ref.at[1]
            else:
                b = _rem(g0, 2)
                gw = _div(g0, 2)
                gprev = _rem(_div(g0 + (2 * NW - 1), 2), NW)
                sl = _rem(_div(g0, NGS), 2)
                s0 = pl.multiple_of(_rem(g0 * GS, HS), GS)
                acc = acc_ref.at[_rem(g0 + 1, 2)]

            def kv_at(buf, h):
                return buf[h // HS, h % HS] if big else buf[sl, s0 + h]

            U = ng * GS
            nq = q_scr.shape[0]
            ss, res = {}, {}
            acc_fresh = False
            for item in _schedule(ng):
                kind, arg = item[:2], item[2:]
                if kind == "QK":
                    h = int(arg)
                    q = q_scr[(h // GS) % nq, :, (h % GS) * Dh:(h % GS + 1) * Dh]
                    ss[h] = jax.lax.dot_general(q, kv_at(k_buf, h), NT, preferred_element_type=f32)
                elif kind == "PV":
                    h = int(arg)
                    pb, part = softmax_unnorm(ss.pop(h))
                    o = jnp.dot(pb, kv_at(v_buf, h), preferred_element_type=f32)
                    if h >= U - GS:
                        o_scr[h - (U - GS)] = o
                        l_scr[h - (U - GS)] = part
                    else:
                        res[h] = (o, part)
                elif kind == "QP":
                    if big:
                        q_proj(b, int(arg), int(arg) % nq)
                    else:
                        q_proj(b, gw, 0)
                elif kind == "SY":
                    k_slot_copy(b, 1).wait()
                    v_slot_copy(b, 1).wait()

                    @pl.when(b + 2 < B)
                    def _():
                        x_copy(b + 2).start()

                    @pl.when(b + 1 < B)
                    def _():
                        k_slot_copy(b + 1, 0).start()
                        v_slot_copy(b + 1, 0).start()
                elif arg == "p":
                    a = acc[...] + o_proj([normalize(o_scr[j], l_scr[j]) for j in range(GS)], gprev)
                    o_ref[0] = a.astype(o_ref.dtype)
                    if big:
                        acc_fresh = True
                    else:
                        acc[...] = a
                else:
                    n, i = int(item[1]), int(arg)
                    r = o_proj([normalize(*res.pop(i * GS + j)) for j in range(n * GS)], i)
                    if acc_fresh:
                        acc[...] = r
                        acc_fresh = False
                    else:
                        acc[...] += r

        def first_starts(groups):
            for gi in groups:
                ck, cv = kv_group_copy(gi, True)
                ck.start()
                cv.start()
                if gi == 1:
                    x_copy(1).start()
                if gi % 2 == 1:
                    wo_copy((gi - 1) // 2).start()
                elif gi > 0:
                    wq_copy(gi // 2).start()

        @pl.when(t < 1)
        def _():
            x_copy(0).start()
            wq_copy(0).start()
            wo_buf[NW - 1] = jnp.zeros((W, D), bf16)

        @pl.when(t == 0)
        def _():
            first_starts(range(0, 1))
            acc_ref[0] = jnp.zeros((Sq, D), f32)

        @pl.when(t <= 0)
        def _():
            first_starts(range(1, 3))
            acc_ref[1] = jnp.zeros((Sq, D), f32)

        @pl.when(t + 1 == 1)
        def _():
            first_starts(range(3, PD))
            o_scr[...] = jnp.zeros_like(o_scr)
            l_scr[...] = jnp.ones_like(l_scr)

        @pl.when(t < NF)
        def _():
            g0 = t
            g_odd = _rem(g0, 2) == 1

            @pl.when(g0 < 2)
            def _():
                x_copy(g0).wait()

            @pl.when(jnp.logical_not(g_odd))
            def _():
                wq_copy(_div(g0, 2)).wait()

            @pl.when(g_odd)
            def _():
                wo_copy(_div(g0 - 1, 2)).wait()

            ck, cv = kv_group_copy(g0, True)
            ck.wait()
            cv.wait()
            body(g0, 1)

            gp = g0 + PD

            @pl.when(gp < NF)
            def _():
                ck, cv = kv_group_copy(gp, True)
                ck.start()
                cv.start()

            @pl.when(jnp.logical_and(gp >= NF, gp < NF + NGS))
            def _():
                ck, cv = kv_group_copy(gp, False)
                ck.start()
                cv.start()

            gp_odd = _rem(gp, 2) == 1

            @pl.when(jnp.logical_and(jnp.logical_not(gp_odd), gp < NF))
            def _():
                wq_copy(_div(gp, 2)).start()

            @pl.when(jnp.logical_and(gp_odd, gp < NF))
            def _():
                wo_copy(_div(gp - 1, 2)).start()

            @pl.when(g0 == X2S)
            def _():
                x_copy(2).start()

            @pl.when(g0 == X2S + 2)
            def _():
                x_copy(3).start()

            @pl.when(g0 == NF - 1)
            def _():
                k_slot_copy(2, 1).start()
                v_slot_copy(2, 1).start()

        @pl.when(jnp.logical_and(t >= NF, t < T - 1))
        def _():
            b = 2 + (t - NF)
            x_copy(b).wait()
            k_slot_copy(b, 0).wait()
            v_slot_copy(b, 0).wait()
            body(b * NW, NW)

            @pl.when(b + 1 < B)
            def _():
                k_slot_copy(b + 1, 1).start()
                v_slot_copy(b + 1, 1).start()

        @pl.when(t == T - 1)
        def _():
            a = acc_ref[1] + o_proj([normalize(o_scr[j], l_scr[j]) for j in range(GS)], NW - 1)
            o_ref[0] = a.astype(o_ref.dtype)

    def out_index(t):
        return (jnp.where(t < NF, 0, jnp.minimum(t - NF + 1, B - 1)), 0, 0)

    any_spec = pl.BlockSpec(memory_space=pl.ANY)
    return pl.pallas_call(
        kernel,
        grid=(T,),
        in_specs=[any_spec] * 5,
        out_specs=pl.BlockSpec((1, Sq, D), out_index),
        out_shape=jax.ShapeDtypeStruct((B, Sq, D), x.dtype),
        scratch_shapes=[
            pltpu.VMEM((2, Sq, D), f32),
            pltpu.VMEM((4, Sq, W), bf16),
            pltpu.VMEM((GS, Sq, Dh), f32),
            pltpu.VMEM((GS, Sq, Dh), f32),
            pltpu.VMEM((B, Sq, D), bf16),
            pltpu.VMEM((2, HS, Sk, Dh), bf16),
            pltpu.VMEM((2, HS, Sk, Dh), bf16),
            pltpu.VMEM((NW, D, W), bf16),
            pltpu.VMEM((NW, W, D), bf16),
            pltpu.SemaphoreType.DMA((2 * NGS,)),
            pltpu.SemaphoreType.DMA((2 * NGS,)),
            pltpu.SemaphoreType.DMA((2,)),
            pltpu.SemaphoreType.DMA((2,)),
            pltpu.SemaphoreType.DMA((NW,)),
            pltpu.SemaphoreType.DMA((NW,)),
            pltpu.SemaphoreType.DMA((2,)),
        ],
        compiler_params=pltpu.CompilerParams(
            dimension_semantics=("arbitrary",),
            vmem_limit_bytes=100 * 1024 * 1024,
            disable_bounds_checks=True,
        ),
        name="gqa_block_cached",
    )(x, kf, vf, wq, wo)
```

```python
import jax
import jax.numpy as jnp
from jax.experimental import pallas as pl
from jax.experimental.pallas import tpu as pltpu

LOG2E = 1.4426950408889634
NT = (((1,), (1,)), ((), ()))
f32 = jnp.float32
bf16 = jnp.bfloat16
GS = 4
HS = 16


def _schedule(ng):
    if ng == 1:
        return "QP0 QK0 OPp QK1 PV0 QK2 PV1 QK3 PV2 PV3".split()
    assert ng == 8 and HS == 16 and GS == 4
    extra = [("QP1", "QK3"), ("OPp", "QK4"), ("QP2", "QK7"), ("O20", "QK11"), ("QP3", "QK11"),
             ("O22", "QK19"), ("QP5", "QK19"), ("QP6", "QK23"), ("O24", "QK26"), ("QP7", "QK27"),
             ("O16", "QK30")]
    s = []
    for h0 in (0, HS):
        dots = ["SY"] if h0 else []
        dots += [f"QP{h0 // GS}", f"QK{h0}"]
        for h in range(h0, h0 + HS):
            dots += [f"QK{h + 1}"] if h + 1 < h0 + HS else []
            dots += [f"PV{h}"]
        for d in dots:
            s += [item for item, before in extra if before == d] + [d]
    return s


def _rem(a, b):
    assert b & (b - 1) == 0
    return a % b if isinstance(a, int) else jax.lax.bitwise_and(a, jnp.int32(b - 1))


def _div(a, b):
    assert b & (b - 1) == 0
    return a // b if isinstance(a, int) else jax.lax.shift_right_logical(a, jnp.int32(b.bit_length() - 1))


@jax.jit
def pallas_standalone__gqa_block_cached__near_ridge_kernel(x, k_cache, v_cache, wq, wo):
    B, Sq, D = x.shape
    _, H, Sk, Dh = k_cache.shape
    assert wq.shape == (D, H * Dh) and wo.shape == (H * Dh, D)
    assert H == 2 * HS and B >= 4 and Dh == 128
    NW = H // GS
    NGS = HS // GS
    NF = 2 * NW
    NM = B - 2
    T = NF + NM + 1
    PD = NGS + 1
    X2S = NW
    c = (Dh ** -0.5) * LOG2E
    nt = Sk // Dh
    W = GS * Dh
    kf = k_cache.reshape(B * H, Sk, Dh)
    vf = v_cache.reshape(B * H, Sk, Dh)

    def kernel(x_hbm, k_hbm, v_hbm, wq_hbm, wo_hbm, out_hbm,
               acc_ref, q_scr, o_scr, l_scr, x_buf, k_buf, v_buf, wq_buf, wo_buf, out_buf,
               sem_fk, sem_fv, sem_mk, sem_mv, sem_wq, sem_wo, sem_x, sem_out):
        t = pl.program_id(0)

        def kv_group_copy(gam, fine):
            if isinstance(gam, int):
                h0 = (gam & 1) * H + (gam >> 1) * GS if gam < NF else gam * GS
            else:
                h0 = jnp.where(gam < NF, _rem(gam, 2) * H + _div(gam, 2) * GS, gam * GS)
            sl = _rem(_div(gam, NGS), 2)
            s0 = _rem(gam * GS, HS)
            if not isinstance(s0, int):
                s0 = pl.multiple_of(s0, GS)
            kd, vd = k_buf.at[sl, pl.ds(s0, GS)], v_buf.at[sl, pl.ds(s0, GS)]
            if fine:
                i = _rem(gam, 2 * NGS)
                sk, sv = sem_fk.at[i], sem_fv.at[i]
            else:
                sk, sv = sem_mk.at[sl], sem_mv.at[sl]
            return (pltpu.make_async_copy(k_hbm.at[pl.ds(h0, GS)], kd, sk),
                    pltpu.make_async_copy(v_hbm.at[pl.ds(h0, GS)], vd, sv))

        def k_slot_copy(b, sl):
            return pltpu.make_async_copy(k_hbm.at[pl.ds(b * H + sl * HS, HS)], k_buf.at[sl], sem_mk.at[sl])

        def v_slot_copy(b, sl):
            return pltpu.make_async_copy(v_hbm.at[pl.ds(b * H + sl * HS, HS)], v_buf.at[sl], sem_mv.at[sl])

        def wq_copy(gi):
            return pltpu.make_async_copy(wq_hbm.at[:, pl.ds(gi * W, W)], wq_buf.at[gi], sem_wq.at[gi])

        def wo_copy(gi):
            return pltpu.make_async_copy(wo_hbm.at[pl.ds(gi * W, W), :], wo_buf.at[gi], sem_wo.at[gi])

        def x_copy(b):
            return pltpu.make_async_copy(x_hbm.at[b], x_buf.at[b], sem_x.at[_rem(b, 2)])

        def out_copy(b):
            sl = _rem(b, 2)
            return pltpu.make_async_copy(out_buf.at[sl], out_hbm.at[b], sem_out.at[sl])

        def softmax_unnorm(s):
            m = jnp.max(s, axis=-1, keepdims=True)
            p = jnp.exp2(s - m)
            ps = [p[:, j * 128:(j + 1) * 128] for j in range(nt)]
            part = ps[0]
            for j in range(1, nt):
                part = part + ps[j]
                if j == 3 or j == nt - 1:
                    ps[j] = jnp.minimum(ps[j], part)
            return jnp.concatenate(ps, axis=-1).astype(bf16), part

        def normalize(o, part):
            l = jnp.sum(part, axis=-1, keepdims=True)
            inv = pl.reciprocal(l, approx=True)
            inv = inv * (2.0 - l * inv)
            return o * inv

        def q_proj(b, gw, slot):
            q = jnp.dot(x_buf[b], wq_buf[gw], preferred_element_type=f32)
            q_scr[slot] = (q * c).astype(bf16)

        def o_proj(ons, gw):
            n = len(ons) // GS
            o_all = jnp.concatenate(ons, axis=-1).astype(bf16)
            w = wo_buf[gw] if n == 1 else wo_buf[pl.ds(gw, n)].reshape(n * W, D)
            return jnp.dot(o_all, w, preferred_element_type=f32)

        def body(g0, ng):
            big = ng == NW
            if big:
                b = _div(g0, NW)
                gprev = NW - 1
                acc = acc_ref.at[1]
            else:
                b = _rem(g0, 2)
                gw = _div(g0, 2)
                gprev = _rem(_div(g0 + (2 * NW - 1), 2), NW)
                sl = _rem(_div(g0, NGS), 2)
                s0 = pl.multiple_of(_rem(g0 * GS, HS), GS)
                acc = acc_ref.at[_rem(g0 + 1, 2)]

            def kv_at(buf, h):
                return buf[h // HS, h % HS] if big else buf[sl, s0 + h]

            U = ng * GS
            nq = q_scr.shape[0]
            ss, res = {}, {}
            acc_fresh = False
            for item in _schedule(ng):
                kind, arg = item[:2], item[2:]
                if kind == "QK":
                    h = int(arg)
                    q = q_scr[(h // GS) % nq, :, (h % GS) * Dh:(h % GS + 1) * Dh]
                    ss[h] = jax.lax.dot_general(q, kv_at(k_buf, h), NT, preferred_element_type=f32)
                elif kind == "PV":
                    h = int(arg)
                    pb, part = softmax_unnorm(ss.pop(h))
                    o = jnp.dot(pb, kv_at(v_buf, h), preferred_element_type=f32)
                    if h >= U - GS:
                        o_scr[h - (U - GS)] = o
                        l_scr[h - (U - GS)] = part
                    else:
                        res[h] = (o, part)
                elif kind == "QP":
                    if big:
                        q_proj(b, int(arg), int(arg) % nq)
                    else:
                        q_proj(b, gw, 0)
                elif kind == "SY":
                    k_slot_copy(b, 1).wait()
                    v_slot_copy(b, 1).wait()

                    @pl.when(b + 2 < B)
                    def _():
                        x_copy(b + 2).start()

                    @pl.when(b + 1 < B)
                    def _():
                        k_slot_copy(b + 1, 0).start()
                        v_slot_copy(b + 1, 0).start()
                elif arg == "p":
                    a = acc[...] + o_proj([normalize(o_scr[j], l_scr[j]) for j in range(GS)], gprev)
                    if big:
                        out_buf[_rem(b - 1, 2)] = a.astype(bf16)
                        out_copy(b - 1).start()
                        acc_fresh = True
                    else:
                        acc[...] = a
                else:
                    n, i = int(item[1]), int(arg)
                    r = o_proj([normalize(*res.pop(i * GS + j)) for j in range(n * GS)], i)
                    if acc_fresh:
                        acc[...] = r
                        acc_fresh = False
                    else:
                        acc[...] += r

        def first_starts(groups):
            for gi in groups:
                ck, cv = kv_group_copy(gi, True)
                ck.start()
                cv.start()
                if gi == 1:
                    x_copy(1).start()
                if gi % 2 == 1:
                    wo_copy((gi - 1) // 2).start()
                elif gi > 0:
                    wq_copy(gi // 2).start()

        def prologue():
            @pl.when(t < 1)
            def _():
                x_copy(0).start()
                wq_copy(0).start()
                wo_buf[NW - 1] = jnp.zeros((W, D), bf16)

            @pl.when(t <= 0)
            def _():
                first_starts(range(0, 1))
                acc_ref[0] = jnp.zeros((Sq, D), f32)

            @pl.when(t + 1 == 1)
            def _():
                first_starts(range(1, 3))
                acc_ref[1] = jnp.zeros((Sq, D), f32)

            @pl.when(t + 2 < 3)
            def _():
                first_starts(range(3, PD))
                o_scr[...] = jnp.zeros_like(o_scr)
                l_scr[...] = jnp.ones_like(l_scr)

        @pl.when(t < NF)
        def _():
            pl.when(t == 0)(prologue)
            g0 = t
            g_odd = _rem(g0, 2) == 1

            @pl.when(g0 < 2)
            def _():
                x_copy(g0).wait()

            @pl.when(jnp.logical_not(g_odd))
            def _():
                wq_copy(_div(g0, 2)).wait()

            @pl.when(g_odd)
            def _():
                wo_copy(_div(g0 - 1, 2)).wait()

            ck, cv = kv_group_copy(g0, True)
            ck.wait()
            cv.wait()
            body(g0, 1)

            gp = g0 + PD

            @pl.when(gp < NF)
            def _():
                ck, cv = kv_group_copy(gp, True)
                ck.start()
                cv.start()

            @pl.when(jnp.logical_and(gp >= NF, gp < NF + NGS))
            def _():
                ck, cv = kv_group_copy(gp, False)
                ck.start()
                cv.start()

            gp_odd = _rem(gp, 2) == 1

            @pl.when(jnp.logical_and(jnp.logical_not(gp_odd), gp < NF))
            def _():
                wq_copy(_div(gp, 2)).start()

            @pl.when(jnp.logical_and(gp_odd, gp < NF))
            def _():
                wo_copy(_div(gp - 1, 2)).start()

            @pl.when(g0 == X2S)
            def _():
                x_copy(2).start()

            @pl.when(g0 == X2S + 2)
            def _():
                x_copy(3).start()

            @pl.when(g0 == NF - 1)
            def _():
                k_slot_copy(2, 1).start()
                v_slot_copy(2, 1).start()
                out_buf[0] = acc_ref[0].astype(bf16)
                out_copy(0).start()

        @pl.when(jnp.logical_and(t >= NF, t < T - 1))
        def _():
            b = 2 + (t - NF)

            @pl.when(b >= 3)
            def _():
                out_copy(b - 3).wait()

            x_copy(b).wait()
            k_slot_copy(b, 0).wait()
            v_slot_copy(b, 0).wait()
            body(b * NW, NW)

            @pl.when(b + 1 < B)
            def _():
                k_slot_copy(b + 1, 1).start()
                v_slot_copy(b + 1, 1).start()

        @pl.when(t == T - 1)
        def _():
            out_copy(B - 3).wait()
            a = acc_ref[1] + o_proj([normalize(o_scr[j], l_scr[j]) for j in range(GS)], NW - 1)
            out_buf[(B - 1) % 2] = a.astype(bf16)
            out_copy(B - 1).start()
            out_copy(B - 2).wait()
            out_copy(B - 1).wait()

    any_spec = pl.BlockSpec(memory_space=pl.ANY)
    return pl.pallas_call(
        kernel,
        grid=(T,),
        in_specs=[any_spec] * 5,
        out_specs=any_spec,
        out_shape=jax.ShapeDtypeStruct((B, Sq, D), x.dtype),
        scratch_shapes=[
            pltpu.VMEM((2, Sq, D), f32),
            pltpu.VMEM((4, Sq, W), bf16),
            pltpu.VMEM((GS, Sq, Dh), f32),
            pltpu.VMEM((GS, Sq, Dh), f32),
            pltpu.VMEM((B, Sq, D), bf16),
            pltpu.VMEM((2, HS, Sk, Dh), bf16),
            pltpu.VMEM((2, HS, Sk, Dh), bf16),
            pltpu.VMEM((NW, D, W), bf16),
            pltpu.VMEM((NW, W, D), bf16),
            pltpu.VMEM((2, Sq, D), bf16),
            pltpu.SemaphoreType.DMA((2 * NGS,)),
            pltpu.SemaphoreType.DMA((2 * NGS,)),
            pltpu.SemaphoreType.DMA((2,)),
            pltpu.SemaphoreType.DMA((2,)),
            pltpu.SemaphoreType.DMA((NW,)),
            pltpu.SemaphoreType.DMA((NW,)),
            pltpu.SemaphoreType.DMA((2,)),
            pltpu.SemaphoreType.DMA((2,)),
        ],
        compiler_params=pltpu.CompilerParams(
            dimension_semantics=("arbitrary",),
            vmem_limit_bytes=100 * 1024 * 1024,
            disable_bounds_checks=True,
        ),
        name="gqa_block_cached",
    )(x, kf, vf, wq, wo)
```

```python
import jax
import jax.numpy as jnp
from jax.experimental import pallas as pl
from jax.experimental.pallas import tpu as pltpu

LOG2E = 1.4426950408889634
NT = (((1,), (1,)), ((), ()))
f32 = jnp.float32
bf16 = jnp.bfloat16
GS = 4
HS = 16


def _schedule(ng):
    if ng == 1:
        return "QP0 QK0 OPp QK1 PV0 QK2 PV1 QK3 PV2 PV3".split()
    assert ng == 8 and HS == 16 and GS == 4
    extra = [("QP1", "QK3"), ("OPp", "QK4"), ("QP2", "QK7"), ("O20", "QK11"), ("QP3", "QK11"),
             ("O22", "QK19"), ("QP5", "QK19"), ("QP6", "QK23"), ("O24", "QK26"), ("QP7", "QK27"),
             ("O16", "QK30")]
    s = []
    for h0 in (0, HS):
        dots = ["SY"] if h0 else []
        dots += [f"QP{h0 // GS}", f"QK{h0}"]
        for h in range(h0, h0 + HS):
            dots += [f"QK{h + 1}"] if h + 1 < h0 + HS else []
            dots += [f"PV{h}"]
        for d in dots:
            s += [item for item, before in extra if before == d] + [d]
    return s


def _rem(a, b):
    assert b & (b - 1) == 0
    return a % b if isinstance(a, int) else jax.lax.bitwise_and(a, jnp.int32(b - 1))


def _div(a, b):
    assert b & (b - 1) == 0
    return a // b if isinstance(a, int) else jax.lax.shift_right_logical(a, jnp.int32(b.bit_length() - 1))


@jax.jit
def pallas_standalone__gqa_block_cached__near_ridge_kernel(x, k_cache, v_cache, wq, wo):
    B, Sq, D = x.shape
    _, H, Sk, Dh = k_cache.shape
    assert wq.shape == (D, H * Dh) and wo.shape == (H * Dh, D)
    assert H == 2 * HS and B >= 4 and Dh == 128 and D % 128 == 0
    NW = H // GS
    NGS = HS // GS
    NF = 2 * NW
    NM = B - 2
    T = NF + NM + 1
    PD = NGS + 1
    X2S = NW
    c = (Dh ** -0.5) * LOG2E
    nt = Sk // Dh
    W = GS * Dh
    kf = k_cache.reshape(B * H, Sk, Dh)
    vf = v_cache.reshape(B * H, Sk, Dh)

    def kernel(x_hbm, k_hbm, v_hbm, wq_hbm, wo_hbm, out_hbm,
               acc_ref, q_scr, o_scr, l_scr, x_buf, k_buf, v_buf, wq_buf, wo_buf, out_buf,
               sem_fk, sem_fv, sem_mk, sem_mv, sem_wq, sem_wo, sem_x, sem_out):
        t = pl.program_id(0)

        def kv_group_copy(gam, fine):
            if isinstance(gam, int):
                h0 = (gam & 1) * H + (gam >> 1) * GS if gam < NF else gam * GS
            else:
                h0 = jnp.where(gam < NF, _rem(gam, 2) * H + _div(gam, 2) * GS, gam * GS)
            sl = _rem(_div(gam, NGS), 2)
            s0 = _rem(gam * GS, HS)
            if not isinstance(s0, int):
                s0 = pl.multiple_of(s0, GS)
            kd, vd = k_buf.at[sl, pl.ds(s0, GS)], v_buf.at[sl, pl.ds(s0, GS)]
            if fine:
                i = _rem(gam, 2 * NGS)
                sk, sv = sem_fk.at[i], sem_fv.at[i]
            else:
                sk, sv = sem_mk.at[sl], sem_mv.at[sl]
            return (pltpu.make_async_copy(k_hbm.at[pl.ds(h0, GS)], kd, sk),
                    pltpu.make_async_copy(v_hbm.at[pl.ds(h0, GS)], vd, sv))

        def k_slot_copy(b, sl):
            return pltpu.make_async_copy(k_hbm.at[pl.ds(b * H + sl * HS, HS)], k_buf.at[sl], sem_mk.at[sl])

        def v_slot_copy(b, sl):
            return pltpu.make_async_copy(v_hbm.at[pl.ds(b * H + sl * HS, HS)], v_buf.at[sl], sem_mv.at[sl])

        def wq_copy(gi):
            return pltpu.make_async_copy(wq_hbm.at[:, pl.ds(gi * W, W)], wq_buf.at[gi], sem_wq.at[gi])

        def wo_copy(gi):
            return pltpu.make_async_copy(wo_hbm.at[pl.ds(gi * W, W), :], wo_buf.at[gi], sem_wo.at[gi])

        def x_copy(b):
            return pltpu.make_async_copy(x_hbm.at[b], x_buf.at[b], sem_x.at[_rem(b, 2)])

        def out_copy(b):
            sl = _rem(b, 2)
            return pltpu.make_async_copy(out_buf.at[sl], out_hbm.at[b], sem_out.at[sl])

        def softmax_unnorm(s):
            m = jnp.max(s, axis=-1, keepdims=True)
            p = jnp.exp2(s - m)
            ps = [p[:, j * 128:(j + 1) * 128] for j in range(nt)]
            part = ps[0]
            for j in range(1, nt):
                part = part + ps[j]
                if j == 3 or j == nt - 1:
                    ps[j] = jnp.minimum(ps[j], part)
            return jnp.concatenate(ps, axis=-1).astype(bf16), part

        def normalize(o, part):
            l = jnp.sum(part, axis=-1, keepdims=True)
            inv = pl.reciprocal(l, approx=True)
            inv = inv * (2.0 - l * inv)
            return o * inv

        def q_proj(b, gw, slot):
            q = jnp.dot(x_buf[b], wq_buf[gw], preferred_element_type=f32)
            q_scr[slot] = (q * c).astype(bf16)

        def o_proj(ons, gw):
            n = len(ons) // GS
            o_all = jnp.concatenate(ons, axis=-1).astype(bf16)
            w = wo_buf[gw] if n == 1 else wo_buf[pl.ds(gw, n)].reshape(n * W, D)
            return jnp.dot(o_all, w, preferred_element_type=f32)

        def body(g0, ng):
            big = ng == NW
            if big:
                b = _div(g0, NW)
                gprev = NW - 1
                acc = acc_ref.at[1]
            else:
                b = _rem(g0, 2)
                gw = _div(g0, 2)
                gprev = _rem(_div(g0 + (2 * NW - 1), 2), NW)
                sl = _rem(_div(g0, NGS), 2)
                s0 = pl.multiple_of(_rem(g0 * GS, HS), GS)
                acc = acc_ref.at[_rem(g0 + 1, 2)]

            def kv_at(buf, h):
                return buf[h // HS, h % HS] if big else buf[sl, s0 + h]

            U = ng * GS
            nq = q_scr.shape[0]
            ss, res = {}, {}
            acc_fresh = False
            for item in _schedule(ng):
                kind, arg = item[:2], item[2:]
                if kind == "QK":
                    h = int(arg)
                    q = q_scr[(h // GS) % nq, :, (h % GS) * Dh:(h % GS + 1) * Dh]
                    ss[h] = jax.lax.dot_general(q, kv_at(k_buf, h), NT, preferred_element_type=f32)
                elif kind == "PV":
                    h = int(arg)
                    pb, part = softmax_unnorm(ss.pop(h))
                    o = jnp.dot(pb, kv_at(v_buf, h), preferred_element_type=f32)
                    if h >= U - GS:
                        o_scr[h - (U - GS)] = o
                        l_scr[h - (U - GS)] = part
                    else:
                        res[h] = (o, part)
                elif kind == "QP":
                    if big:
                        q_proj(b, int(arg), int(arg) % nq)
                    else:
                        q_proj(b, gw, 0)
                elif kind == "SY":
                    k_slot_copy(b, 1).wait()
                    v_slot_copy(b, 1).wait()

                    @pl.when(b + 2 < B)
                    def _():
                        x_copy(b + 2).start()

                    @pl.when(b + 1 < B)
                    def _():
                        k_slot_copy(b + 1, 0).start()
                        v_slot_copy(b + 1, 0).start()
                elif arg == "p":
                    a = acc[...] + o_proj([normalize(o_scr[j], l_scr[j]) for j in range(GS)], gprev)
                    if big:
                        out_buf[_rem(b - 1, 2)] = a.astype(bf16)
                        out_copy(b - 1).start()
                        acc_fresh = True
                    else:
                        acc[...] = a
                else:
                    n, i = int(item[1]), int(arg)
                    r = o_proj([normalize(*res.pop(i * GS + j)) for j in range(n * GS)], i)
                    if acc_fresh:
                        acc[...] = r
                        acc_fresh = False
                    else:
                        acc[...] += r

        def first_starts(groups):
            for gi in groups:
                ck, cv = kv_group_copy(gi, True)
                ck.start()
                cv.start()
                if gi == 1:
                    x_copy(1).start()
                if gi % 2 == 1:
                    wo_copy((gi - 1) // 2).start()
                elif gi > 0:
                    wq_copy(gi // 2).start()

        def prologue():
            @pl.when(t < 1)
            def _():
                x_copy(0).start()
                wq_copy(0).start()
                wo_buf[NW - 1] = jnp.zeros((W, D), bf16)

            @pl.when(t <= 0)
            def _():
                first_starts(range(0, 1))
                acc_ref[0] = jnp.zeros((Sq, D), f32)

            @pl.when(t + 1 == 1)
            def _():
                first_starts(range(1, 3))
                acc_ref[1] = jnp.zeros((Sq, D), f32)

            @pl.when(t + 2 < 3)
            def _():
                first_starts(range(3, PD))
                o_scr[...] = jnp.zeros_like(o_scr)
                l_scr[...] = jnp.ones_like(l_scr)

        @pl.when(t < NF)
        def _():
            pl.when(t == 0)(prologue)
            g0 = t
            g_odd = _rem(g0, 2) == 1

            @pl.when(g0 < 2)
            def _():
                x_copy(g0).wait()

            @pl.when(jnp.logical_not(g_odd))
            def _():
                wq_copy(_div(g0, 2)).wait()

            @pl.when(g_odd)
            def _():
                wo_copy(_div(g0 - 1, 2)).wait()

            ck, cv = kv_group_copy(g0, True)
            ck.wait()
            cv.wait()
            body(g0, 1)

            gp = g0 + PD

            @pl.when(gp < NF)
            def _():
                ck, cv = kv_group_copy(gp, True)
                ck.start()
                cv.start()

            @pl.when(jnp.logical_and(gp >= NF, gp < NF + NGS))
            def _():
                ck, cv = kv_group_copy(gp, False)
                ck.start()
                cv.start()

            gp_odd = _rem(gp, 2) == 1

            @pl.when(jnp.logical_and(jnp.logical_not(gp_odd), gp < NF))
            def _():
                wq_copy(_div(gp, 2)).start()

            @pl.when(jnp.logical_and(gp_odd, gp < NF))
            def _():
                wo_copy(_div(gp - 1, 2)).start()

            @pl.when(g0 == X2S)
            def _():
                x_copy(2).start()

            @pl.when(g0 == X2S + 2)
            def _():
                x_copy(3).start()

            @pl.when(g0 == NF - 1)
            def _():
                k_slot_copy(2, 1).start()
                v_slot_copy(2, 1).start()
                out_buf[0] = acc_ref[0].astype(bf16)
                out_copy(0).start()

        @pl.when(jnp.logical_and(t >= NF, t < T - 1))
        def _():
            b = 2 + (t - NF)

            @pl.when(b >= 3)
            def _():
                out_copy(b - 3).wait()

            x_copy(b).wait()
            k_slot_copy(b, 0).wait()
            v_slot_copy(b, 0).wait()
            body(b * NW, NW)

            @pl.when(b + 1 < B)
            def _():
                k_slot_copy(b + 1, 1).start()
                v_slot_copy(b + 1, 1).start()

        @pl.when(t == T - 1)
        def _():
            out_copy(B - 3).wait()
            a = acc_ref[1] + o_proj([normalize(o_scr[j], l_scr[j]) for j in range(GS)], NW - 1)
            sl = (B - 1) % 2
            copies = []
            for j in range(D // 128):
                cols = pl.ds(j * 128, 128)
                out_buf[sl, :, cols] = a[:, j * 128:(j + 1) * 128].astype(bf16)
                cp = pltpu.make_async_copy(out_buf.at[sl, :, cols], out_hbm.at[B - 1, :, cols], sem_out.at[sl])
                cp.start()
                copies.append(cp)
            out_copy(B - 2).wait()
            for cp in copies:
                cp.wait()

    any_spec = pl.BlockSpec(memory_space=pl.ANY)
    return pl.pallas_call(
        kernel,
        grid=(T,),
        in_specs=[any_spec] * 5,
        out_specs=any_spec,
        out_shape=jax.ShapeDtypeStruct((B, Sq, D), x.dtype),
        scratch_shapes=[
            pltpu.VMEM((2, Sq, D), f32),
            pltpu.VMEM((4, Sq, W), bf16),
            pltpu.VMEM((GS, Sq, Dh), f32),
            pltpu.VMEM((GS, Sq, Dh), f32),
            pltpu.VMEM((B, Sq, D), bf16),
            pltpu.VMEM((2, HS, Sk, Dh), bf16),
            pltpu.VMEM((2, HS, Sk, Dh), bf16),
            pltpu.VMEM((NW, D, W), bf16),
            pltpu.VMEM((NW, W, D), bf16),
            pltpu.VMEM((2, Sq, D), bf16),
            pltpu.SemaphoreType.DMA((2 * NGS,)),
            pltpu.SemaphoreType.DMA((2 * NGS,)),
            pltpu.SemaphoreType.DMA((2,)),
            pltpu.SemaphoreType.DMA((2,)),
            pltpu.SemaphoreType.DMA((NW,)),
            pltpu.SemaphoreType.DMA((NW,)),
            pltpu.SemaphoreType.DMA((2,)),
            pltpu.SemaphoreType.DMA((2,)),
        ],
        compiler_params=pltpu.CompilerParams(
            dimension_semantics=("arbitrary",),
            vmem_limit_bytes=100 * 1024 * 1024,
            disable_bounds_checks=True,
        ),
        name="gqa_block_cached",
    )(x, kf, vf, wq, wo)
```
